```python
import jax
import jax.numpy as jnp

def _softmax(x, axis=-1):
    return jax.nn.softmax(x, axis=axis)
def _gelu(x):
    return jax.nn.gelu(x, approximate=True)
def _silu(x):
    return jax.nn.silu(x)
def _sigmoid(x):
    return jax.nn.sigmoid(x)
def _layernorm(x, axis=-1, eps=1e-5):
    m = jnp.mean(x, axis=axis, keepdims=True)
    v = jnp.var(x, axis=axis, keepdims=True)
    return (x - m) / jnp.sqrt(v + eps)
def _scatter_add(tgt, idx, src, axis=0):
    return tgt.at[idx].add(src)
def _segment_sum(src, seg, n):
    return jax.ops.segment_sum(src, seg, n)
class _Rng:
    def __init__(self, key):
        self._k = key
    def _next(self):
        self._k, sub = jax.random.split(self._k)
        return sub
    def normal(self, shape):
        return jax.random.normal(self._next(), shape, dtype=jnp.bfloat16)
    def randint(self, lo, hi, shape):
        return jax.random.randint(self._next(), shape, lo, hi, dtype=jnp.int32)
    def uniform(self, shape, lo=0.0, hi=1.0):
        return jax.random.uniform(self._next(), shape, jnp.bfloat16, lo, hi)
    def permutation(self, n):
        return jax.random.permutation(self._next(), n)


kernel_name = 'gated_mix__ssm_conv_h3__compressed_kv_cla__prompt'

def setup_inputs():
    _rng = _Rng(jax.random.key(int.from_bytes(__import__("os").urandom(4), "little")))
    _w = (lambda a: (lambda t: t.astype(jnp.bfloat16) if jnp.issubdtype(t.dtype, jnp.floating) else t)(jnp.asarray(a)))
    def _A_setup():
        B, S, D = 1, 2048, 1024
        ks = 4
        return {
            "q": _w((lambda *s: _rng.normal(s) * 0.05)(B, S, D)),
            "k": _w((lambda *s: _rng.normal(s) * 0.05)(B, S, D)),
            "v": _w((lambda *s: _rng.normal(s) * 0.05)(B, S, D)),
            "shift_k": _w((lambda *s: _rng.normal(s) * 0.05)(D, ks) * 0.5),
            "ssm_k": _w((lambda *s: _rng.normal(s) * 0.05)(D, S) * (1.0 / S ** 0.5)),
            "ssm_D": _w((lambda *s: _rng.normal(s) * 0.05)(D)),
        }
    _A_in = _A_setup()

    def _B_setup():
        B, H, Sq, Sk, D, M = 1, 32, 2048, 2048, 128, 1024
        Dc = 4 * D
        return {
            "x": _w((lambda *s: _rng.normal(s) * 0.05)(B, Sq, M)),
            "c_kv": _w((lambda *s: _rng.normal(s) * 0.05)(B, Sk, Dc)),
            "w_q": _w((lambda *s: _rng.normal(s) * 0.05)(M, H, D) * (M ** -0.5)),
            "w_uk": _w((lambda *s: _rng.normal(s) * 0.05)(Dc, H, D) * (Dc ** -0.5)),
            "w_uv": _w((lambda *s: _rng.normal(s) * 0.05)(Dc, H, D) * (Dc ** -0.5)),
            "w_o": _w((lambda *s: _rng.normal(s) * 0.05)(H, D, M) * ((H * D) ** -0.5)),
        }
    _B_in = _B_setup()

    return {
        "A_q": _A_in["q"],
        "A_k": _A_in["k"],
        "A_v": _A_in["v"],
        "A_shift_k": _A_in["shift_k"],
        "A_ssm_k": _A_in["ssm_k"],
        "A_ssm_D": _A_in["ssm_D"],
        "B_x": _B_in["x"],
        "B_c_kv": _B_in["c_kv"],
        "B_w_q": _B_in["w_q"],
        "B_w_uk": _B_in["w_uk"],
        "B_w_uv": _B_in["w_uv"],
        "B_w_o": _B_in["w_o"],
        "gate_w": _w((lambda *s: _rng.normal(s) * 0.05)(1024)),
    }

def reference(A_q, A_k, A_v, A_shift_k, A_ssm_k, A_ssm_D, B_x, B_c_kv, B_w_q, B_w_uk, B_w_uv, B_w_o, gate_w):
    def _A_ref(q, k, v, shift_k, ssm_k, ssm_D):
        B, S, D = q.shape
        ks = shift_k.shape[-1]
        k_pad = jnp.pad(k, ((0, 0), (ks - 1, 0), (0, 0)))
        k_shift = jnp.zeros_like(k)
        for t in range(ks):
            k_shift = k_shift + k_pad[:, t:t + S, :] * shift_k[:, ks - 1 - t][None, None, :]
        kv = k_shift * v
        L = 2 * S
        kv_pad = jnp.pad(kv, ((0, 0), (0, S), (0, 0)))
        kf_pad = jnp.pad(ssm_k, ((0, 0), (0, S)))
        kv_f = (lambda x, axes=(-2,-1): jnp.fft.rfft2(x.astype(jnp.float32), axes=axes))(kv_pad[:, None, :, :], axes=(1, 2))
        kf_f = (lambda x, axes=(-2,-1): jnp.fft.rfft2(x.astype(jnp.float32), axes=axes))(kf_pad[:, None, :], axes=(1, 2))
        kf_f = (lambda x, *d: x.transpose(*d))(kf_f, 1, 2, 0)
        y_f = kv_f * kf_f[None, :, :, :]
        y = (lambda x, s, axes=(-2,-1): jnp.fft.irfft2(x, s=s, axes=axes).astype(jnp.bfloat16))(y_f, (1, L), axes=(1, 2))[:, 0, :S, :]
        y = y + kv * ssm_D[None, None, :]
        return q * y

    def _B_ref(x, c_kv, w_q, w_uk, w_uv, w_o):
        B, Sq, M = x.shape[0], x.shape[1], x.shape[2]
        Sk = c_kv.shape[1]
        H, D = w_q.shape[1], w_q.shape[2]
        q = jnp.einsum("bqm,mhd->bhqd", x, w_q)
        k = jnp.einsum("bkc,chd->bhkd", c_kv, w_uk)
        v = jnp.einsum("bkc,chd->bhkd", c_kv, w_uv)
        scores = jnp.einsum("bhqd,bhkd->bhqk", q, k) * (D ** -0.5)
        off = Sk - Sq
        qi = jnp.arange(Sq)[:, None]
        kj = jnp.arange(Sk)[None, :]
        cmask = kj <= (qi + off)
        scores = jnp.where(cmask[None, None], scores, -1e9)
        p = _softmax(scores, axis=-1)
        ctx = jnp.einsum("bhqk,bhkd->bhqd", p, v)
        return jnp.einsum("bhqd,hdm->bqm", ctx, w_o)

    x = A_q
    g = _sigmoid((x * gate_w).sum(-1, keepdims=True))
    a = _A_ref(x, A_k, A_v, A_shift_k, A_ssm_k, A_ssm_D)
    b = _B_ref(x, B_c_kv, B_w_q, B_w_uk, B_w_uv, B_w_o)
    return g * a + (1 - g) * b
```

```python
import functools
import jax
import jax.numpy as jnp
import numpy as np
from jax import lax
from jax.experimental import pallas as pl
from jax.experimental.pallas import tpu as pltpu

S = 2048
H = 32
DH = 128
M = 1024
DC = 512
C = 128
NC = S // C
NDT = M // C
NEG = -1e9
LOG2E = 1.4426950408889634

NT = (((1,), (1,)), ((), ()))


def _dft_matrix():
    k = np.concatenate([np.arange(0, C, 2), np.arange(1, C, 2)]).astype(np.float64)
    t = np.arange(C, dtype=np.float64)
    th = 2.0 * np.pi * (k[:, None] + 0.5) * t[None, :] / (2 * C)
    return np.concatenate([np.cos(th), -np.sin(th)], axis=0)


def _pair_weights(w_ref, grp, p, rows):
    n = rows * (H // 2) - (H // 2 - 4)
    w32 = w_ref.bitcast(jnp.uint32).at[pl.ds(pl.multiple_of(grp * 4, 4), n), :]
    w = w32[pl.ds(p, rows, stride=H // 2), :]
    lo = pltpu.unpack_elementwise(w, index=0, packed_dtype=jnp.bfloat16, unpacked_dtype=jnp.float32)
    hi = pltpu.unpack_elementwise(w, index=1, packed_dtype=jnp.bfloat16, unpacked_dtype=jnp.float32)
    return lo.astype(jnp.bfloat16), hi.astype(jnp.bfloat16)


def _kernel(x_ref, c_ref, wq_ref, wuk_ref, wuv_ref, wo_ref, aq_ref, ak_ref, av_ref, aqg_ref,
            sk_ref, ssm_ref, d_ref, gw_ref, f_ref, g_ref, o_ref,
            wq_s, wk_s, wv_s, q_s, k_s, v_s, ctx_s, gate_s, s_s, p_s, xf_s, hf_s, z_s, *, TQ):
    i = pl.program_id(0)

    for p in range(4):
        @pl.when((i < H) & ((i & 7) == 2 * p))
        def _(p=p):
            grp = lax.shift_right_logical(i, 3)
            for w_ref, w_s, rows in ((wq_ref, wq_s, M), (wuk_ref, wk_s, DC), (wuv_ref, wv_s, DC)):
                lo, hi = _pair_weights(w_ref, grp, p, rows)
                w_s[0] = lo
                w_s[1] = hi

    @pl.when(i < H)
    def _attn():
        h = i
        wq = wq_s[h & 1]
        wk = wk_s[h & 1]
        wv = wv_s[h & 1]
        q = jnp.dot(x_ref[...], wq, preferred_element_type=jnp.float32) * (DH ** -0.5 * LOG2E)
        q_s[...] = q.astype(jnp.bfloat16)
        c = c_ref[...]
        k_s[...] = jnp.dot(c, wk, preferred_element_type=jnp.float32).astype(jnp.bfloat16)
        v_s[...] = jnp.dot(c, wv, preferred_element_type=jnp.float32).astype(jnp.bfloat16)
        gl = jnp.sum(aqg_ref[...].astype(jnp.float32) * gw_ref[...].astype(jnp.float32).reshape(1, M), axis=-1, keepdims=True)
        gate_s[pl.ds(pl.multiple_of(h * (S // H), S // H), S // H), :] = jnp.broadcast_to(jax.nn.sigmoid(gl), (S // H, C))
        ri = lax.broadcasted_iota(jnp.int32, (TQ, TQ), 0)
        ci = lax.broadcasted_iota(jnp.int32, (TQ, TQ), 1)
        for b in range(S // TQ):
            n = (b + 1) * TQ
            qb = q_s[b * TQ:(b + 1) * TQ, :]
            s = lax.dot_general(qb, k_s[0:n, :], NT, preferred_element_type=jnp.float32)
            sd = jnp.where(ci <= ri, s[:, n - TQ:], NEG)
            s = sd if b == 0 else jnp.concatenate([s[:, :n - TQ], sd], axis=1)
            m = jnp.max(s, axis=-1, keepdims=True)
            p = jnp.exp2(s - m)
            l = jnp.sum(p, axis=-1, keepdims=True)
            o = jnp.dot(p.astype(jnp.bfloat16), v_s[0:n, :], preferred_element_type=jnp.float32)
            ctx_s[h, b * TQ:(b + 1) * TQ, :] = (o / l).astype(jnp.bfloat16)

    @pl.when(i >= H)
    def _mix():
        j = i - H
        f32 = jnp.float32
        kk = ak_ref[...].astype(f32)
        sk = sk_ref[...].astype(f32)
        row = lax.broadcasted_iota(jnp.int32, (S, C), 0)
        ks = kk * sk[0:1, :]
        for t in range(1, 4):
            sh = jnp.where(row >= t, pltpu.roll(kk, t, 0), 0.0)
            ks = ks + sh * sk[t:t + 1, :]
        kv = (ks * av_ref[...].astype(f32)).astype(jnp.bfloat16)
        F = f_ref[...]
        for a in range(NC):
            xf_s[a] = jnp.dot(F, kv[a * C:(a + 1) * C, :], preferred_element_type=f32)
        prev = None
        for a in range(NC):
            hm = lax.dot_general(F, ssm_ref[:, a * C:(a + 1) * C], NT, preferred_element_type=f32)
            if prev is None:
                hf_s[a] = hm
            else:
                hf_s[a, 0:64] = hm[0:64] - prev[128:192]
                hf_s[a, 64:128] = hm[64:128] + prev[192:256]
                hf_s[a, 128:192] = hm[128:192] + prev[0:64]
                hf_s[a, 192:256] = hm[192:256] - prev[64:128]
            prev = hm
        R = 16
        for fr in range(C // R):
            re = slice(fr * R, (fr + 1) * R)
            im = slice(C + fr * R, C + (fr + 1) * R)
            for a in range(NC):
                zr = zi = None
                for b in range(a + 1):
                    xr, xi = xf_s[b, re], xf_s[b, im]
                    hr, hi = hf_s[a - b, re], hf_s[a - b, im]
                    tr = xr * hr - xi * hi
                    ti = xr * hi + xi * hr
                    zr = tr if zr is None else zr + tr
                    zi = ti if zi is None else zi + ti
                z_s[a, re] = zr.astype(jnp.bfloat16)
                z_s[a, im] = zi.astype(jnp.bfloat16)
        G = g_ref[...]
        dd = d_ref[...].astype(f32).reshape(NDT, C)
        dsel = jnp.sum(jnp.where(lax.broadcasted_iota(jnp.int32, (NDT, C), 0) == j, dd, 0.0), axis=0, keepdims=True)
        acc = None
        for h in range(H):
            t = jnp.dot(ctx_s[h], wo_ref[h * DH:(h + 1) * DH, :], preferred_element_type=f32)
            acc = t if acc is None else acc + t
        for a in range(NC):
            rs = slice(a * C, (a + 1) * C)
            y = jnp.dot(G, z_s[a], preferred_element_type=f32) * (1.0 / C) + kv[rs].astype(f32) * dsel
            g = gate_s[rs, :]
            o_ref[rs, :] = (g * (aq_ref[rs, :].astype(f32) * y) + (1.0 - g) * acc[rs]).astype(o_ref.dtype)


@jax.jit
def pallas_gated_mix__ssm_conv_h3__compressed_kv_cla__prompt_kernel(A_q, A_k, A_v, A_shift_k, A_ssm_k, A_ssm_D, B_x, B_c_kv, B_w_q, B_w_uk, B_w_uv, B_w_o, gate_w):
    TQ = 256
    bf = jnp.bfloat16
    F = _dft_matrix()
    f_np = F.astype(bf)
    g_np = np.ascontiguousarray(F.T).astype(bf)
    one = pl.Buffered(1)
    dt = lambda i: jnp.maximum(i - H, 0)
    full = lambda shape: pl.BlockSpec(shape, lambda i: (0,) * len(shape), pipeline_mode=one)
    col = lambda rows: pl.BlockSpec((rows, C), lambda i: (0, dt(i)))
    aq = A_q.reshape(S, M)
    out = pl.pallas_call(
        functools.partial(_kernel, TQ=TQ),
        grid=(H + NDT,),
        in_specs=[
            full((S, M)), full((S, DC)), full((M * H, DH)), full((DC * H, DH)), full((DC * H, DH)),
            col(H * DH), col(S), col(S), col(S),
            pl.BlockSpec((S // H, M), lambda i: (jnp.minimum(i, H - 1), 0)),
            col(4),
            pl.BlockSpec((C, S), lambda i: (dt(i), 0)),
            full((M,)), full((M,)), full((2 * C, C)), full((C, 2 * C)),
        ],
        out_specs=col(S),
        out_shape=jax.ShapeDtypeStruct((S, M), bf),
        scratch_shapes=[
            pltpu.VMEM((2, M, DH), bf), pltpu.VMEM((2, DC, DH), bf), pltpu.VMEM((2, DC, DH), bf),
            pltpu.VMEM((S, DH), bf), pltpu.VMEM((S, DH), bf), pltpu.VMEM((S, DH), bf),
            pltpu.VMEM((H, S, DH), bf), pltpu.VMEM((S, C), jnp.float32),
            pltpu.VMEM((TQ, S), jnp.float32), pltpu.VMEM((TQ, S), bf),
            pltpu.VMEM((NC, 2 * C, C), jnp.float32), pltpu.VMEM((NC, 2 * C, C), jnp.float32),
            pltpu.VMEM((NC, 2 * C, C), bf),
        ],
        compiler_params=pltpu.CompilerParams(dimension_semantics=("arbitrary",), vmem_limit_bytes=100 * 1024 * 1024),
        name="fused",
    )(aq, B_c_kv.reshape(S, DC), B_w_q.reshape(M * H, DH), B_w_uk.reshape(DC * H, DH),
      B_w_uv.reshape(DC * H, DH), B_w_o.reshape(H * DH, M), aq, A_k.reshape(S, M), A_v.reshape(S, M), aq,
      A_shift_k.T, A_ssm_k, A_ssm_D, gate_w, f_np, g_np)
    return out.reshape(1, S, M)
```

```python
import functools
import os
import jax
import jax.numpy as jnp
import numpy as np
from jax import lax
from jax.experimental import pallas as pl
from jax.experimental.pallas import tpu as pltpu

S = 2048
H = 32
DH = 128
M = 1024
DC = 512
C = 128
NC = S // C
NDT = M // C
TQ = 256
NEG = -1e9
LOG2E = 1.4426950408889634
NT = (((1,), (1,)), ((), ()))
f32 = jnp.float32
bf16 = jnp.bfloat16
u32 = jnp.uint32
THROTTLE = int(os.environ.get("THROTTLE", "0"))
NWIN = int(os.environ.get("NWIN", "52"))
SR = int(os.environ.get("SR", "32"))
PULL = int(os.environ.get("PULL", "0"))
PR = int(os.environ.get("PR", "256"))
NB = int(os.environ.get("NB", "4"))
HG = int(os.environ.get("HG", "4"))


def _dft_matrices():
    k = np.concatenate([np.arange(0, C, 2), np.arange(1, C, 2)]).astype(np.float64)
    t = np.arange(C, dtype=np.float64)
    th = 2.0 * np.pi * (k[:, None] + 0.5) * t[None, :] / (2 * C)
    fwd = np.concatenate([np.cos(th), -np.sin(th)], axis=0)
    inv = np.stack([np.cos(th), -np.sin(th)], axis=1).reshape(2 * C, C).T
    return fwd, np.ascontiguousarray(inv)


def _dot(a, b):
    return jnp.dot(a, b, preferred_element_type=f32)


def _rows(w):
    return pltpu.bitcast(w, bf16)


def _words(x):
    return pltpu.bitcast(x.astype(bf16), u32)


def _recip(l):
    r = pl.reciprocal(l, approx=True)
    return r * (2.0 - l * r)


def _kernel(x_hbm, c_hbm, wq_hbm, wuk_hbm, wuv_hbm, wo_hbm, ak_hbm, av_hbm, sk_hbm, ssm_hbm, d_hbm, gw_hbm,
            f_hbm, g_hbm, o_hbm,
            x_s, c_s, wq_b, wk_b, wv_b, wo_b, akv_b, ssm_b, o_b, sk_s, d_s, gw_s, f_s, g_s,
            kt_s, v_s, ctx_s, gate_s, sf_s, a_s, b_s,
            sem_in, sem_x, sem_c, sem_w, sem_t, sem_o, *, phases):

    def pair_copies(p, slot):
        return [pltpu.make_async_copy(w.bitcast(u32).at[:, p], b.at[slot], sem_w.at[n, slot])
                for n, (w, b) in enumerate(((wuk_hbm, wk_b), (wuv_hbm, wv_b), (wq_hbm, wq_b)))]

    def tile_copies(j, slot):
        col = pl.ds(pl.multiple_of(j * C, C), C)
        return [pltpu.make_async_copy(src, dst, sem_t.at[n, slot])
                for n, (src, dst) in enumerate(((ssm_hbm.at[col, :], ssm_b.at[slot]),
                                                (ak_hbm.bitcast(u32).at[:, col], akv_b.at[slot, 0]),
                                                (av_hbm.bitcast(u32).at[:, col], akv_b.at[slot, 1]),
                                                (wo_hbm.bitcast(u32).at[:, col], wo_b.at[slot])))]

    def out_copy(j, slot):
        return pltpu.make_async_copy(o_b.at[slot], o_hbm.at[:, pl.ds(pl.multiple_of(j * C, C), C)], sem_o.at[slot])

    c_cp = [pltpu.make_async_copy(c_hbm.bitcast(u32).at[:, n * C:(n + 1) * C], c_s.at[n], sem_c.at[n])
            for n in range(DC // C)]
    x_cp = [pltpu.make_async_copy(x_hbm.bitcast(u32).at[:, n * C:(n + 1) * C], x_s.at[n], sem_x.at[n])
            for n in range(M // C)]
    small = [pltpu.make_async_copy(s, d, sem_in.at[n]) for n, (s, d) in enumerate((
        (gw_hbm, gw_s), (sk_hbm, sk_s), (d_hbm, d_s), (f_hbm.bitcast(u32), f_s), (g_hbm, g_s)))]
    for cp in c_cp + pair_copies(0, 0) + x_cp + small:
        cp.start()
    for cp in c_cp + x_cp + small:
        cp.wait()

    def head(h, carry):
        slot = lax.shift_right_logical(h, 1) & 1

        @pl.when((h & 1) == 0)
        def _():
            p = lax.shift_right_logical(h, 1)
            for cp in pair_copies(p, slot):
                cp.wait()

            @pl.when(p + 1 < H // 2)
            def _():
                for cp in pair_copies(p + 1, 1 - slot):
                    cp.start()

            @pl.when(p == 1)
            def _():
                for cp in tile_copies(0, 0):
                    cp.start()

        sh = ((1 - (h & 1)) * 16).astype(u32)

        def weight(b):
            w = lax.shift_left(b[slot], sh) & jnp.uint32(0xFFFF0000)
            return pltpu.bitcast(w, f32).astype(bf16)

        def latent():
            return jnp.concatenate([_rows(c_s[n]) for n in range(DC // C)], axis=1)

        wk = weight(wk_b)
        kt_s[...] = pltpu.bitcast(_dot(latent(), wk).astype(bf16).T, u32)
        rows = pl.ds(pl.multiple_of(h * (S // H // 2), S // H // 2), S // H // 2)
        xg = jnp.concatenate([_rows(x_s[n, rows, :]) for n in range(M // C)], axis=1)
        gl = jnp.sum(xg.astype(f32) * gw_s[...].astype(f32).reshape(1, M), axis=-1, keepdims=True)
        gate_s[pl.ds(pl.multiple_of(h * (S // H), S // H), S // H), :] = jnp.broadcast_to(jax.nn.sigmoid(gl), (S // H, C))
        wq = weight(wq_b)
        tri = lax.broadcasted_iota(jnp.int32, (C, C), 1) <= lax.broadcasted_iota(jnp.int32, (C, C), 0)

        def scores(b):
            r0 = b * TQ
            n1 = r0 + C
            xb = jnp.concatenate([_rows(x_s[n, r0 // 2:(r0 + TQ) // 2, :]) for n in range(M // C)], axis=1)
            q = _dot(xb, wq) * (DH ** -0.5 * LOG2E)
            s1 = _dot(q.astype(bf16), _rows(kt_s[:, 0:n1]))
            s2 = _dot(q[C:].astype(bf16), _rows(kt_s[:, n1:n1 + C]))
            return s1, s2

        def softmax(b, s1, s2):
            r0 = b * TQ
            top = jnp.where(tri, s1[:C, r0:], NEG)
            if b > 0:
                top = jnp.concatenate([s1[:C, :r0], top], axis=1)
            bot = jnp.concatenate([s1[C:], jnp.where(tri, s2, NEG)], axis=1)
            pt = jnp.exp2(top - jnp.max(top, axis=-1, keepdims=True))
            pb = jnp.exp2(bot - jnp.max(bot, axis=-1, keepdims=True))
            lt = jnp.sum(pt, axis=-1, keepdims=True)
            lb = jnp.sum(pb, axis=-1, keepdims=True)
            p1 = jnp.concatenate([pt, pb[:, :r0 + C]], axis=0).astype(bf16)
            return p1, pb[:, r0 + C:].astype(bf16), _recip(lt), _recip(lb)

        def values(b, p1, p2, lt, lb):
            r0 = b * TQ
            n1 = r0 + C
            o = _dot(p1, _rows(v_s[0:n1 // 2, :]))
            ob = o[C:] + _dot(p2, _rows(v_s[n1 // 2:(n1 + C) // 2, :]))
            ctx_s[h, r0 // 2:(r0 + C) // 2, :] = _words(o[:C] * lt)
            ctx_s[h, (r0 + C) // 2:(r0 + TQ) // 2, :] = _words(ob * lb)

        nb = S // TQ
        s_cur = scores(nb - 1)
        v_s[...] = _words(_dot(latent(), weight(wv_b)))
        for b in range(nb - 1, -1, -1):
            s_next = scores(b - 1) if b > 0 else None
            p = softmax(b, *s_cur)
            values(b, *p)
            s_cur = s_next
        return carry

    if phases & 1:
        lax.fori_loop(0, H, head, 0)

    def mix(j, carry):
        slot = j & 1
        for cp in tile_copies(j, slot):
            cp.wait()

        @pl.when(j + 1 < NDT)
        def _():
            for cp in tile_copies(j + 1, 1 - slot):
                cp.start()

        @pl.when(j >= 2)
        def _():
            out_copy(j - 2, slot).wait()

        col = pl.ds(pl.multiple_of(j * C, C), C)
        zero = lax.shift_right_logical(j, 5)
        Z0, KV, PAD = H + zero, H + 2 + zero, H + 3 + zero
        last = None
        prev = None
        for a in range(NC):
            hm = lax.dot_general(_rows(f_s[...]), ssm_b[slot, :, a * C:(a + 1) * C], NT, preferred_element_type=f32)
            ha = NC + a + zero
            if prev is None:
                sf_s[ha] = hm
            else:
                sf_s[ha, 0:64] = hm[0:64] - prev[128:192]
                sf_s[ha, 64:128] = hm[64:128] + prev[192:256]
                sf_s[ha, 128:192] = hm[128:192] + prev[0:64]
                sf_s[ha, 192:256] = hm[192:256] - prev[64:128]
            prev = hm
            if a == NC - 4:
                last = hm

        sk = sk_s[:, col].astype(f32)
        dd = d_s[...].astype(f32).reshape(NDT, C)
        dsel = jnp.sum(jnp.where(lax.broadcasted_iota(jnp.int32, (NDT, C), 0) == j, dd, 0.0), axis=0, keepdims=True)

        def release_kv(t):
            akv_b[slot + zero, 2, 0:8] = pltpu.bitcast(t, u32)

        def release_sf(t):
            sf_s[2 * NC + zero, 0:8] = t

        def short_steps():
            R = SR
            for n in range(S // R):
                if n == 0:
                    kk = _rows(akv_b[slot, 0, 0:R // 2]).astype(f32)
                    kk = jnp.concatenate([jnp.zeros((8, C), f32), kk], axis=0)
                else:
                    kk = _rows(akv_b[slot, 0, n * R // 2 - 8:(n + 1) * R // 2]).astype(f32)[8:]
                ks = kk[8:] * sk[0:1, :]
                for t in range(1, 4):
                    ks = ks + pltpu.roll(kk, t, 0)[8:] * sk[t:t + 1, :]
                ws = slice(n * R // 2, (n + 1) * R // 2)
                ctx_s[KV, ws] = _words(ks * _rows(akv_b[slot, 1, ws]).astype(f32))
                yield

        done = [0]
        pending = []

        def branch_a(blk):
            for a in range(blk * NB, (blk + 1) * NB):
                ws = slice(a * C // 2, (a + 1) * C // 2)
                rs = slice(a * C, (a + 1) * C)
                z = _rows(ctx_s[Z0 + a // 8, (a % 8) * C:(a % 8 + 1) * C])
                y = _dot(g_s[...], z) * (1.0 / C) + _rows(ctx_s[KV, ws]).astype(f32) * dsel
                av = gate_s[rs, :] * (_rows(x_s[j, ws, :]).astype(f32) * y)
                if a * C // PR in pending:
                    o_b[slot, rs, :] = (av + b_s[rs, :]).astype(bf16)
                    if (a + 1) * C % PR == 0:
                        pending.remove(a * C // PR)
                else:
                    a_s[rs, :] = av
                done[0] = (a + 1) * C

        ready = []

        def conv_steps():
            for blk in range(NC // NB):
                outs = range(blk * NB, (blk + 1) * NB)
                for fr in range(C // 8):
                    re = slice(fr * 8, (fr + 1) * 8)
                    im = slice(C + fr * 8, C + (fr + 1) * 8)
                    hs = {}
                    z = {}
                    for b in range(outs[-1], -1, -1):
                        xr, xi = sf_s[b, re], sf_s[b, im]
                        for a in outs:
                            if a < b:
                                continue
                            if a - b not in hs:
                                hs[a - b] = (sf_s[NC + a - b, re], sf_s[NC + a - b, im])
                            hr, hi = hs[a - b]
                            tr = xr * hr - xi * hi
                            ti = xr * hi + xi * hr
                            z[a] = (tr, ti) if a not in z else (z[a][0] + tr, z[a][1] + ti)
                        if b == 0:
                            for a in outs:
                                ctx_s[Z0 + a // 8, (a % 8) * C + fr * 8:(a % 8) * C + fr * 8 + 8] = (
                                    pltpu.pack_elementwise(list(z[a]), packed_dtype=bf16))
                            if fr == C // 8 - 1:
                                ready.append(blk)
                            yield None
                        else:
                            yield [z[outs[-1]][1], z[outs[-1]][0]][:PULL]

        NG = H // HG
        SL = PR // 32
        state = dict(prev=last, points=0, conv=0, short=0)
        sgen, cgen = short_steps(), conv_steps()
        nconv = (C // 8) * sum((blk + 1) * NB for blk in range(NC // NB))
        nshort = S // SR

        def proj(r):
            acc = None
            for g in range(NG):
                parts = []
                for i in range(SL):
                    rel = state["prev"][32 * i:32 * i + 8]
                    if r == 0:
                        want = -(-(g * SL + i + 1) * nshort // (NG * SL - SL))
                        want = min(want, nshort)
                        if want > state["short"]:
                            release_kv(rel)
                            while state["short"] < want:
                                next(sgen)
                                state["short"] += 1
                    else:
                        state["points"] += 1
                        want = min(nconv, -(-state["points"] * nconv // (NWIN * SL)))
                        if want > state["conv"]:
                            release_sf(rel)
                            while state["conv"] < want:
                                pull = next(cgen)
                                state["conv"] += 1
                            for n, pv in enumerate(pull or ()):
                                ctx_s[PAD, 8 * n:8 * n + 8] = pltpu.bitcast(pv, u32)
                    w0 = (r * PR + 32 * i) // 2
                    parts.append(jnp.concatenate([_rows(ctx_s[h, w0:w0 + 16]) for h in range(g * HG, (g + 1) * HG)], axis=1))
                lhs = jnp.concatenate(parts, axis=0)
                t = _dot(lhs, _rows(wo_b[slot, g * HG * DH // 2:(g + 1) * HG * DH // 2, :]))
                state["prev"] = t
                acc = t if acc is None else acc + t
                while ready:
                    branch_a(ready.pop(0))
            return acc

        for r in range(S // PR):
            acc = proj(r)
            if r == 0:
                for a in range(NC):
                    xm = _dot(_rows(f_s[...]), _rows(ctx_s[KV, a * C // 2:(a + 1) * C // 2]))
                    sf_s[a + zero] = xm
                state["prev"] = xm
            rs = slice(r * PR, (r + 1) * PR)
            if done[0] >= (r + 1) * PR:
                o_b[slot, rs, :] = (a_s[rs, :] + (1.0 - gate_s[rs, :]) * acc).astype(bf16)
            else:
                b_s[rs, :] = (1.0 - gate_s[rs, :]) * acc
                pending.append(r)
        assert not pending and state["conv"] == nconv and state["short"] == nshort
        out_copy(j, slot).start()
        return carry

    if phases & 2:
        lax.fori_loop(0, NDT, mix, 0)
        out_copy(NDT - 2, 0).wait()
        out_copy(NDT - 1, 1).wait()


def make(phases=3):
    @jax.jit
    def fn(A_q, A_k, A_v, A_shift_k, A_ssm_k, A_ssm_D, B_x, B_c_kv, B_w_q, B_w_uk, B_w_uv, B_w_o, gate_w):
        fwd, inv = _dft_matrices()
        V = pltpu.VMEM
        out = pl.pallas_call(
            functools.partial(_kernel, phases=phases),
            in_specs=[pl.BlockSpec(memory_space=pl.ANY)] * 14,
            out_specs=pl.BlockSpec(memory_space=pl.ANY),
            out_shape=jax.ShapeDtypeStruct((S, M), bf16),
            scratch_shapes=[
                V((M // C, S // 2, C), u32), V((DC // C, S // 2, C), u32),
                V((2, M, DH), u32), V((2, DC, DH), u32), V((2, DC, DH), u32),
                V((2, H * DH // 2, C), u32), V((2, 3, S // 2, C), u32), V((2, C, S), bf16),
                V((2, S, C), bf16),
                V((4, M), bf16), V((M,), bf16), V((M,), bf16), V((C, C), u32), V((C, 2 * C), bf16),
                V((DH // 2, S), u32), V((S // 2, DH), u32),
                V((H + 4, S // 2, DH), u32), V((S, C), f32),
                V((2 * NC + 1, 2 * C, C), f32), V((S, C), f32), V((S, C), f32),
                pltpu.SemaphoreType.DMA((5,)), pltpu.SemaphoreType.DMA((M // C,)), pltpu.SemaphoreType.DMA((DC // C,)),
                pltpu.SemaphoreType.DMA((3, 2)), pltpu.SemaphoreType.DMA((4, 2)), pltpu.SemaphoreType.DMA((2,)),
            ],
            compiler_params=pltpu.CompilerParams(vmem_limit_bytes=100 * 1024 * 1024),
            name="fused",
        )(A_q.reshape(S, M), B_c_kv.reshape(S, DC), B_w_q, B_w_uk, B_w_uv, B_w_o.reshape(H * DH, M),
          A_k.reshape(S, M), A_v.reshape(S, M), A_shift_k.T, A_ssm_k, A_ssm_D, gate_w,
          fwd.astype(bf16), inv.astype(bf16))
        return out.reshape(1, S, M)
    return fn


pallas_gated_mix__ssm_conv_h3__compressed_kv_cla__prompt_kernel = make(3)
```

```python
import functools
import jax
import jax.numpy as jnp
import numpy as np
from jax import lax
from jax.experimental import pallas as pl
from jax.experimental.pallas import tpu as pltpu

S = 2048
H = 32
DH = 128
M = 1024
DC = 512
C = 128
NC = S // C
NDT = M // C
TQ = 256
KT = H + 3
NEG = -1e9
LOG2E = 1.4426950408889634
NT = (((1,), (1,)), ((), ()))
f32 = jnp.float32
bf16 = jnp.bfloat16
u32 = jnp.uint32
NWIN = 52
SR = 32
PR = 256
XS = 0
RP = 32
CG = 4
LAG = 2
LATE = 4
UNR = 1
WAITS = {1: {1: (1, 2), 3: (3, 4), 5: (5, 6, 7)}, 2: {b: (b,) for b in range(1, 8)}, 3: {1: (1, 2, 3), 4: (4, 5, 6, 7)}, 4: {1: (1,), 2: (2,), 3: (3,), 4: (4, 5), 6: (6, 7)}}
NB = 4
HG = 4


def _dft_matrices():
    k = np.concatenate([np.arange(0, C, 2), np.arange(1, C, 2)]).astype(np.float64)
    t = np.arange(C, dtype=np.float64)
    th = 2.0 * np.pi * (k[:, None] + 0.5) * t[None, :] / (2 * C)
    fwd = np.concatenate([np.cos(th), -np.sin(th)], axis=0)
    inv = np.stack([np.cos(th), -np.sin(th)], axis=1).reshape(2 * C, C).T
    return fwd, np.ascontiguousarray(inv)


def _dot(a, b):
    return jnp.dot(a, b, preferred_element_type=f32)


def _ld(ref, lead, r0, n):
    w = ref if ref.dtype == u32 else ref.bitcast(u32)
    return pltpu.bitcast(w[(*lead, pl.ds(r0 // 2 if isinstance(r0, int) else r0, n // 2), slice(None))], bf16)


def _recip(l):
    r = pl.reciprocal(l, approx=True)
    return r * (2.0 - l * r)


def _kernel(x_hbm, c_hbm, wq_hbm, wuk_hbm, wuv_hbm, wo_hbm, ak_hbm, av_hbm, sk_hbm, ssm_hbm, d_hbm, gw_hbm,
            f_hbm, g_hbm, o_hbm,
            x_w, c_w, wq_b, wk_b, wv_b, wo_w, akv_w, ssm_w, o_b, sk_s, d_s, gw_s, f_w, g_w,
            w_w, q_s, k_s, kt_s, v_s, res_s, gate_s, sf_s, a_s, b_s,
            sem_in, sem_r, sem_w, sem_t, sem_o, *, phases):

    def pair_copies(p, slot):
        return [pltpu.make_async_copy(w.bitcast(u32).at[:, p], b.at[slot], sem_w.at[n, slot])
                for n, (w, b) in enumerate(((wuk_hbm, wk_b), (wuv_hbm, wv_b), (wq_hbm, wq_b)))]

    def tile_copies(j, slot):
        col = pl.ds(pl.multiple_of(j * C, C), C)
        row = pl.ds(pl.multiple_of(j * (C // 2), C // 2), C // 2)
        return [pltpu.make_async_copy(src, dst, sem_t.at[n, slot])
                for n, (src, dst) in enumerate(((ssm_hbm.bitcast(u32).at[row, :], ssm_w.at[slot]),
                                                (ak_hbm.bitcast(u32).at[:, col], akv_w.at[slot, 0]),
                                                (av_hbm.bitcast(u32).at[:, col], akv_w.at[slot, 1]),
                                                (wo_hbm.bitcast(u32).at[:, col], wo_w.at[slot])))]

    def out_copy(j, slot):
        col = pl.ds(pl.multiple_of(j * C, C), C)
        return pltpu.make_async_copy(o_b.at[slot], o_hbm.at[:, col], sem_o.at[slot])

    row_cp = [[pltpu.make_async_copy(src.bitcast(u32).at[b * TQ // 2:(b + 1) * TQ // 2, :],
                                     dst.at[b * TQ // 2:(b + 1) * TQ // 2, :], sem_r.at[n, b])
               for n, (src, dst) in enumerate(((c_hbm, c_w), (x_hbm, x_w)))] for b in range(S // TQ)]
    small = [pltpu.make_async_copy(s, d, sem_in.at[n]) for n, (s, d) in enumerate((
        (gw_hbm, gw_s), (sk_hbm, sk_s), (d_hbm, d_s), (f_hbm.bitcast(u32), f_w), (g_hbm.bitcast(u32), g_w)))]
    for cp in pair_copies(0, 0) + row_cp[0] + small + sum(row_cp[1:], []):
        cp.start()
    for cp in row_cp[0] + small + ([] if LATE and phases & 1 else sum(row_cp[1:], [])):
        cp.wait()

    def unpack_weights(h):
        slot = lax.shift_right_logical(h, 1) & 1
        sh = ((h & 1) * 16).astype(u32)
        for b, n0, n in ((wk_b, 0, DC), (wv_b, DC, DC), (wq_b, 2 * DC, M)):
            lo = lax.shift_right_logical(b[slot, pl.ds(0, n // 2, stride=2), :], sh) & jnp.uint32(0xFFFF)
            hi = lax.shift_left(b[slot, pl.ds(1, n // 2, stride=2), :], 16 - sh) & jnp.uint32(0xFFFF0000)
            w_w[n0 // 2:(n0 + n) // 2, :] = lo | hi

    def project(b):
        cb = _ld(c_w, (), b * TQ, TQ)
        kv = _dot(cb, jnp.concatenate([_ld(w_w, (), 0, DC), _ld(w_w, (), DC, DC)], axis=1))
        k_s[...] = kv[:, :DH].astype(bf16)
        for t in range(TQ // C):
            kt_s[b * TQ // C + t] = _ld(k_s, (), t * C, C).T
        xb = _ld(x_w, (), b * TQ, TQ)
        q = _dot(xb, _ld(w_w, (), 2 * DC, M)) * (DH ** -0.5 * LOG2E)
        return q, kv[:, DH:]

    def head(h, carry, waits=None):
        p = lax.shift_right_logical(h, 1) + 1

        @pl.when(((h & 1) == 0) & (p < H // 2))
        def _():
            for cp in pair_copies(p, p & 1):
                cp.start()

        @pl.when(((h & 1) == 1) & (p < H // 2))
        def _():
            for cp in pair_copies(p, p & 1):
                cp.wait()

        @pl.when((h == 3) & (phases == 3))
        def _():
            for cp in tile_copies(0, 0):
                cp.start()

        tri = lax.broadcasted_iota(jnp.int32, (C, C), 1) <= lax.broadcasted_iota(jnp.int32, (C, C), 0)

        def scores(b, q, q2):
            r0 = b * TQ
            s1 = _dot(q, jnp.concatenate([_ld(kt_s, (t,), 0, C) for t in range(2 * b + 1)], axis=1))
            s2 = jnp.where(tri, _dot(q2, _ld(kt_s, (2 * b + 1,), 0, C)), NEG)
            diag = jnp.concatenate([jnp.where(tri, s1[:C, r0:], NEG), s1[C:, r0:]], axis=0)
            tiles = [s1[:, t * C:(t + 1) * C] for t in range(2 * b)] + [diag]
            m = functools.reduce(jnp.maximum, tiles)
            m = jnp.concatenate([m[:C], jnp.maximum(m[C:], s2)], axis=0)
            return tiles, s2, jnp.broadcast_to(jnp.max(m, axis=-1, keepdims=True), (TQ, C))

        def values(b, tiles, s2, m):
            r0 = b * TQ
            n1 = r0 + C
            ps = [jnp.exp2(t - m) for t in tiles]
            p2 = jnp.exp2(s2 - m[C:])
            o = _dot(jnp.concatenate(ps, axis=1).astype(bf16), _ld(v_s, (), 0, n1))
            ob = o[C:] + _dot(p2.astype(bf16), _ld(v_s, (), n1, C))
            l = functools.reduce(jnp.add, ps)
            l = jnp.concatenate([l[:C], l[C:] + p2], axis=0)
            l = _recip(jnp.broadcast_to(jnp.sum(l, axis=-1, keepdims=True), (TQ, DH)))
            res_s[h, r0:n1, :] = (o[:C] * l[:C]).astype(bf16)
            res_s[h, n1:n1 + C, :] = (ob * l[C:]).astype(bf16)

        nb = S // TQ
        sm = scores(0, _ld(q_s, (), 0, TQ), _ld(q_s, (), C, C))
        for b in range(1, nb):
            for n in (waits or {}).get(b, ()):
                for cp in row_cp[n]:
                    cp.wait()
            q, v = project(b)
            v_s[b * TQ:(b + 1) * TQ, :] = v.astype(bf16)
            values(b - 1, *sm)
            sm = scores(b, q.astype(bf16), q[C:].astype(bf16))
        rows = pl.ds(pl.multiple_of(h * (S // H), S // H), S // H)
        xg = pltpu.bitcast(x_w[pl.ds(pl.multiple_of(h * (S // H // 2), S // H // 2), S // H // 2), :], bf16)
        gl = jnp.sum(xg.astype(f32) * gw_s[...].astype(f32).reshape(1, M), axis=-1, keepdims=True)
        gate_s[rows, :] = jax.nn.sigmoid(jnp.broadcast_to(gl, (S // H, C)))
        unpack_weights(jnp.minimum(h + 1, H - 1))
        q, v = project(0)
        q_s[...] = q.astype(bf16)
        values(nb - 1, *sm)
        v_s[0:TQ, :] = v.astype(bf16)
        return carry

    if phases & 1:
        for cp in pair_copies(0, 0):
            cp.wait()
        unpack_weights(jnp.int32(0))
        q, v = project(0)
        q_s[...] = q.astype(bf16)
        v_s[0:TQ, :] = v.astype(bf16)
        if LATE:
            head(jnp.int32(0), 0, WAITS[LATE])
        lax.fori_loop(1 if LATE else 0, H, head, 0, unroll=UNR)

    def mix(j, carry):
        slot = j & 1
        for cp in tile_copies(j, slot):
            cp.wait()

        @pl.when(j + 1 < NDT)
        def _():
            for cp in tile_copies(j + 1, 1 - slot):
                cp.start()

        @pl.when(j >= 2)
        def _():
            out_copy(j - 2, slot).wait()

        col = pl.ds(pl.multiple_of(j * C, C), C)
        zero = lax.shift_right_logical(j, 5)
        Z0, KV = H + zero, H + 2 + zero
        last = None
        prev = None
        for a in range(NC):
            hm = lax.dot_general(_ld(f_w, (), 0, 2 * C), pltpu.bitcast(ssm_w[slot, :, a * C:(a + 1) * C], bf16), NT, preferred_element_type=f32)
            ha = NC + a + zero
            if prev is None:
                sf_s[ha] = hm
            else:
                sf_s[ha, 0:64] = hm[0:64] - prev[128:192]
                sf_s[ha, 64:128] = hm[64:128] + prev[192:256]
                sf_s[ha, 128:192] = hm[128:192] + prev[0:64]
                sf_s[ha, 192:256] = hm[192:256] - prev[64:128]
            prev = hm
            if a == NC - 4:
                last = hm

        sk = sk_s[:, col].astype(f32)
        dd = d_s[...].astype(f32).reshape(NDT, C)
        dsel = jnp.sum(jnp.where(lax.broadcasted_iota(jnp.int32, (NDT, C), 0) == j, dd, 0.0), axis=0, keepdims=True)

        def short_steps():
            R = SR
            for n in range(S // R):
                if n == 0:
                    kk = jnp.concatenate([jnp.zeros((8, C), f32), _ld(akv_w, (slot, 0), 0, R).astype(f32)], axis=0)
                else:
                    kk = _ld(akv_w, (slot, 0), n * R - 16, R + 16).astype(f32)[8:]
                ks = kk[8:] * sk[0:1, :]
                for t in range(1, 4):
                    ks = ks + pltpu.roll(kk, t, 0)[8:] * sk[t:t + 1, :]
                rs = slice(n * R, (n + 1) * R)
                res_s[KV, rs] = (ks * _ld(akv_w, (slot, 1), n * R, R).astype(f32)).astype(bf16)
                yield

        done = [0]
        pending = []

        def branch_a(blk):
            for a in range(blk * NB, (blk + 1) * NB):
                rs = slice(a * C, (a + 1) * C)
                z = _ld(res_s, (Z0 + a // 8,), (a % 8) * 2 * C, 2 * C)
                y = _dot(_ld(g_w, (), 0, C), z) * (1.0 / C) + _ld(res_s, (KV,), a * C, C).astype(f32) * dsel
                av = gate_s[rs, :] * (pltpu.bitcast(x_w[a * C // 2:(a + 1) * C // 2, col], bf16).astype(f32) * y)
                if a * C // PR in pending:
                    o_b[slot, rs, :] = (av + b_s[rs, :]).astype(bf16)
                    if (a + 1) * C % PR == 0:
                        pending.remove(a * C // PR)
                else:
                    a_s[rs, :] = av
                done[0] = (a + 1) * C

        ready = []

        def conv_steps():
            for blk in range(NC // NB):
                outs = range(blk * NB, (blk + 1) * NB)
                for fr in range(C // 8):
                    re = slice(fr * 8, (fr + 1) * 8)
                    im = slice(C + fr * 8, C + (fr + 1) * 8)
                    hs = {}
                    z = {}
                    for b in range(outs[-1], -1, -1):
                        xr, xi = sf_s[b, re], sf_s[b, im]
                        for a in outs:
                            if a < b:
                                continue
                            if a - b not in hs:
                                hs[a - b] = (sf_s[NC + a - b, re], sf_s[NC + a - b, im])
                            hr, hi = hs[a - b]
                            tr = xr * hr - xi * hi
                            ti = xr * hi + xi * hr
                            z[a] = (tr, ti) if a not in z else (z[a][0] + tr, z[a][1] + ti)
                        if b == 0:
                            for a in outs:
                                res_s.bitcast(u32)[Z0 + a // 8, (a % 8) * C + fr * 8:(a % 8) * C + fr * 8 + 8] = (
                                    pltpu.pack_elementwise(list(z[a]), packed_dtype=bf16))
                            if fr == C // 8 - 1:
                                ready.append(blk)
                        yield

        NG = H // HG
        SL = PR // 32
        state = dict(prev=last, points=0, conv=0, short=0)
        sgen, cgen = short_steps(), conv_steps()
        nconv = (C // 8) * sum((blk + 1) * NB for blk in range(NC // NB))
        nshort = S // SR

        def proj(r):
            acc = None
            for g in range(NG):
                parts = []
                for i in range(SL):
                    rel = state["prev"][32 * i:32 * i + 8]
                    if r == 0:
                        want = min(nshort, -(-(g * SL + i + 1) * nshort // (NG * SL - SL)))
                        if want > state["short"]:
                            akv_w[slot + zero, 2, 0:8] = pltpu.bitcast(rel, u32)
                            while state["short"] < want:
                                next(sgen)
                                state["short"] += 1
                    else:
                        state["points"] += 1
                        want = min(nconv, -(-state["points"] * nconv // (NWIN * SL)))
                        if want > state["conv"]:
                            sf_s[2 * NC + zero, 0:8] = rel
                            while state["conv"] < want:
                                next(cgen)
                                state["conv"] += 1
                    parts.append(jnp.concatenate(
                        [_ld(res_s, (h,), r * PR + 32 * i, 32) for h in range(g * HG, (g + 1) * HG)], axis=1))
                t = _dot(jnp.concatenate(parts, axis=0), _ld(wo_w, (slot,), g * HG * DH, HG * DH))
                state["prev"] = t
                acc = t if acc is None else acc + t
                while ready:
                    branch_a(ready.pop(0))
            return acc

        for r in range(S // PR):
            acc = proj(r)
            if r == 0:
                for a in range(NC):
                    xm = _dot(_ld(f_w, (), 0, 2 * C), _ld(res_s, (KV,), a * C, C))
                    sf_s[a + zero] = xm
                state["prev"] = xm
            rs = slice(r * PR, (r + 1) * PR)
            if done[0] >= (r + 1) * PR:
                o_b[slot, rs, :] = (a_s[rs, :] + (1.0 - gate_s[rs, :]) * acc).astype(bf16)
            else:
                b_s[rs, :] = (1.0 - gate_s[rs, :]) * acc
                pending.append(r)
        assert not pending and state["conv"] == nconv and state["short"] == nshort
        out_copy(j, slot).start()
        return carry

    if phases & 2:
        lax.fori_loop(0, NDT, mix, 0)
        out_copy(NDT - 2, 0).wait()
        out_copy(NDT - 1, 1).wait()


def make(phases=3):
    @jax.jit
    def fn(A_q, A_k, A_v, A_shift_k, A_ssm_k, A_ssm_D, B_x, B_c_kv, B_w_q, B_w_uk, B_w_uv, B_w_o, gate_w):
        fwd, inv = _dft_matrices()
        V = pltpu.VMEM
        out = pl.pallas_call(
            functools.partial(_kernel, phases=phases),
            in_specs=[pl.BlockSpec(memory_space=pl.ANY)] * 14,
            out_specs=pl.BlockSpec(memory_space=pl.ANY),
            out_shape=jax.ShapeDtypeStruct((S, M), bf16),
            scratch_shapes=[
                V((S // 2, M), u32), V((S // 2, DC), u32),
                V((2, M, DH), u32), V((2, DC, DH), u32), V((2, DC, DH), u32),
                V((2, H * DH // 2, C), u32), V((2, 3, S // 2, C), u32), V((2, C // 2, S), u32),
                V((2, S, C), bf16),
                V((4, M), bf16), V((M,), bf16), V((M,), bf16), V((C, C), u32), V((C // 2, 2 * C), u32),
                V((DC + M // 2, DH), u32), V((TQ, DH), bf16), V((TQ, DH), bf16),
                V((NC, DH, C), bf16), V((S, DH), bf16),
                V((H + 3, S, DH), bf16), V((S, C), f32),
                V((2 * NC + 1, 2 * C, C), f32), V((S, C), f32), V((S, C), f32),
                pltpu.SemaphoreType.DMA((5,)), pltpu.SemaphoreType.DMA((2, S // TQ)),
                pltpu.SemaphoreType.DMA((3, 2)), pltpu.SemaphoreType.DMA((4, 2)), pltpu.SemaphoreType.DMA((2,)),
            ],
            compiler_params=pltpu.CompilerParams(vmem_limit_bytes=100 * 1024 * 1024),
            name="fused",
        )(A_q.reshape(S, M), B_c_kv.reshape(S, DC), B_w_q, B_w_uk, B_w_uv, B_w_o.reshape(H * DH, M),
          A_k.reshape(S, M), A_v.reshape(S, M), A_shift_k.T, A_ssm_k, A_ssm_D, gate_w,
          fwd.astype(bf16), inv.astype(bf16))
        return out.reshape(1, S, M)
    return fn


pallas_gated_mix__ssm_conv_h3__compressed_kv_cla__prompt_kernel = make(3)
```

```python
import functools
import jax
import jax.numpy as jnp
import numpy as np
from jax import lax
from jax.experimental import pallas as pl
from jax.experimental.pallas import tpu as pltpu

S = 2048
H = 32
DH = 128
M = 1024
DC = 512
C = 128
NC = S // C
NDT = M // C
TQ = 256
KT = H + 3
NEG = -1e9
LOG2E = 1.4426950408889634
NT = (((1,), (1,)), ((), ()))
f32 = jnp.float32
bf16 = jnp.bfloat16
u32 = jnp.uint32
NWIN = 52
SR = 32
PR = 256
XS = 0
RP = 32
CG = 4
LAG = 2
LATE = 4
UNR = 1
WAITS = {1: {1: (1, 2), 3: (3, 4), 5: (5, 6, 7)}, 2: {b: (b,) for b in range(1, 8)}, 3: {1: (1, 2, 3), 4: (4, 5, 6, 7)}, 4: {1: (1,), 2: (2,), 3: (3,), 4: (4, 5), 6: (6, 7)}}
PEEL = 1
FIN = [8] * 8
QF = 0
GP = 8
UP = 0
SF = 0
PF = 0
NB = 4
HG = 4


def _dft_matrices():
    k = np.concatenate([np.arange(0, C, 2), np.arange(1, C, 2)]).astype(np.float64)
    t = np.arange(C, dtype=np.float64)
    th = 2.0 * np.pi * (k[:, None] + 0.5) * t[None, :] / (2 * C)
    fwd = np.concatenate([np.cos(th), -np.sin(th)], axis=0)
    inv = np.stack([np.cos(th), -np.sin(th)], axis=1).reshape(2 * C, C).T
    return fwd, np.ascontiguousarray(inv)


def _dot(a, b):
    return jnp.dot(a, b, preferred_element_type=f32)


def _ld(ref, lead, r0, n):
    w = ref if ref.dtype == u32 else ref.bitcast(u32)
    return pltpu.bitcast(w[(*lead, pl.ds(r0 // 2 if isinstance(r0, int) else r0, n // 2), slice(None))], bf16)


def _recip(l):
    r = pl.reciprocal(l, approx=True)
    return r * (2.0 - l * r)


def _kernel(x_hbm, c_hbm, wq_hbm, wuk_hbm, wuv_hbm, wo_hbm, ak_hbm, av_hbm, sk_hbm, ssm_hbm, d_hbm, gw_hbm,
            f_hbm, g_hbm, o_hbm,
            x_w, c_w, wq_b, wk_b, wv_b, wo_w, akv_w, ssm_w, o_b, sk_s, d_s, gw_s, f_w, g_w,
            q_s, k_s, kt_s, v_s, res_s, gate_s, sf_s, a_s, b_s,
            sem_in, sem_r, sem_w, sem_t, sem_o, *, phases):

    def pair_copies(p, slot):
        return [pltpu.make_async_copy(w.bitcast(u32).at[:, p], b.at[slot], sem_w.at[n, slot])
                for n, (w, b) in enumerate(((wuk_hbm, wk_b), (wuv_hbm, wv_b), (wq_hbm, wq_b)))]

    def tile_copies(j, slot):
        col = pl.ds(pl.multiple_of(j * C, C), C)
        row = pl.ds(pl.multiple_of(j * (C // 2), C // 2), C // 2)
        return [pltpu.make_async_copy(src, dst, sem_t.at[n, slot])
                for n, (src, dst) in enumerate(((ssm_hbm.bitcast(u32).at[row, :], ssm_w.at[slot]),
                                                (ak_hbm.bitcast(u32).at[:, col], akv_w.at[slot, 0]),
                                                (av_hbm.bitcast(u32).at[:, col], akv_w.at[slot, 1]),
                                                (wo_hbm.bitcast(u32).at[:, col], wo_w.at[slot])))]

    def out_copy(j, slot):
        col = pl.ds(pl.multiple_of(j * C, C), C)
        return pltpu.make_async_copy(o_b.at[slot], o_hbm.at[:, col], sem_o.at[slot])

    row_cp = [[pltpu.make_async_copy(src.bitcast(u32).at[b * TQ // 2:(b + 1) * TQ // 2, :],
                                     dst.at[b * TQ // 2:(b + 1) * TQ // 2, :], sem_r.at[n, b])
               for n, (src, dst) in enumerate(((c_hbm, c_w), (x_hbm, x_w)))] for b in range(S // TQ)]
    small = [pltpu.make_async_copy(s, d, sem_in.at[n]) for n, (s, d) in enumerate((
        (gw_hbm, gw_s), (sk_hbm, sk_s), (d_hbm, d_s), (f_hbm.bitcast(u32), f_w), (g_hbm.bitcast(u32), g_w)))]
    for cp in pair_copies(0, 0) + row_cp[0] + small + sum(row_cp[1:], []):
        cp.start()
    for cp in row_cp[0] + small + ([] if PEEL and phases & 1 else sum(row_cp[1:], [])):
        cp.wait()

    def unpack_weights(h):
        slot = lax.shift_right_logical(h, 1) & 1
        sh = ((h & 1) * 16).astype(u32)
        for b, n0, n in ((wk_b, 0, DC), (wv_b, DC, DC), (wq_b, 2 * DC, M)):
            w = lax.shift_left(b[slot], 16 - sh) & jnp.uint32(0xFFFF0000)
            res_s[KT, n0:n0 + n, :] = pltpu.bitcast(w, f32).astype(bf16)

    def project(b):
        def queries():
            return _dot(_ld(x_w, (), b * TQ, TQ), _ld(res_s, (KT,), 2 * DC, M)) * (DH ** -0.5 * LOG2E)

        q = queries() if QF else None
        kv = _dot(_ld(c_w, (), b * TQ, TQ),
                  jnp.concatenate([_ld(res_s, (KT,), 0, DC), _ld(res_s, (KT,), DC, DC)], axis=1))
        k_s[...] = kv[:, :DH].astype(bf16)
        for t in range(TQ // C):
            kt_s[b * TQ // C + t] = _ld(k_s, (), t * C, C).T
        return (q if QF else queries()), kv[:, DH:]

    def head(h, carry, waits=None):
        p = lax.shift_right_logical(h, 1) + 1

        @pl.when(((h & 1) == 0) & (p < H // 2))
        def _():
            for cp in pair_copies(p, p & 1):
                cp.start()

        @pl.when(((h & 1) == 1) & (p < H // 2))
        def _():
            for cp in pair_copies(p, p & 1):
                cp.wait()

        tri = lax.broadcasted_iota(jnp.int32, (C, C), 1) <= lax.broadcasted_iota(jnp.int32, (C, C), 0)

        def scores(b, q, q2):
            r0 = b * TQ
            if SF:
                s2 = jnp.where(tri, _dot(q2, _ld(kt_s, (2 * b + 1,), 0, C)), NEG)
            s1 = _dot(q, jnp.concatenate([_ld(kt_s, (t,), 0, C) for t in range(2 * b + 1)], axis=1))
            if not SF:
                s2 = jnp.where(tri, _dot(q2, _ld(kt_s, (2 * b + 1,), 0, C)), NEG)
            diag = jnp.concatenate([jnp.where(tri, s1[:C, r0:], NEG), s1[C:, r0:]], axis=0)
            tiles = [s1[:, t * C:(t + 1) * C] for t in range(2 * b)] + [diag]
            m = functools.reduce(jnp.maximum, tiles)
            m = jnp.concatenate([m[:C], jnp.maximum(m[C:], s2)], axis=0)
            return tiles, s2, jnp.broadcast_to(jnp.max(m, axis=-1, keepdims=True), (TQ, C))

        def values(b, tiles, s2, m):
            r0 = b * TQ
            n1 = r0 + C
            ps = [jnp.exp2(t - m) for t in tiles]
            p2 = jnp.exp2(s2 - m[C:])
            if PF:
                low = _dot(p2.astype(bf16), _ld(v_s, (), n1, C))
            o = _dot(jnp.concatenate(ps, axis=1).astype(bf16), _ld(v_s, (), 0, n1))
            ob = o[C:] + (low if PF else _dot(p2.astype(bf16), _ld(v_s, (), n1, C)))
            l = functools.reduce(jnp.add, ps)
            l = jnp.concatenate([l[:C], l[C:] + p2], axis=0)
            return b, jnp.concatenate([o[:C], ob], axis=0), l

        def finish(b, o, l):
            l = _recip(jnp.broadcast_to(jnp.sum(l, axis=-1, keepdims=True), (TQ, DH)))
            res_s[h, b * TQ:(b + 1) * TQ, :] = (o * l).astype(bf16)

        def gate():
            rows = pl.ds(pl.multiple_of(h * (S // H), S // H), S // H)
            xg = pltpu.bitcast(x_w[pl.ds(pl.multiple_of(h * (S // H // 2), S // H // 2), S // H // 2), :], bf16)
            gl = jnp.sum(xg.astype(f32) * gw_s[...].astype(f32).reshape(1, M), axis=-1, keepdims=True)
            gate_s[rows, :] = jax.nn.sigmoid(jnp.broadcast_to(gl, (S // H, C)))

        nb = S // TQ
        todo = []
        sm = scores(0, _ld(q_s, (), 0, TQ), _ld(q_s, (), C, C))
        for b in range(1, nb):
            for n in (waits or {}).get(b, ()):
                for cp in row_cp[n]:
                    cp.wait()
            q, v = project(b)
            v_s[b * TQ:(b + 1) * TQ, :] = v.astype(bf16)
            if GP == b:
                gate()
            if b == nb - 1 and UP == 1:
                unpack_weights(jnp.minimum(h + 1, H - 1))
            todo.append(values(b - 1, *sm))
            if b == nb - 1 and UP == 2:
                unpack_weights(jnp.minimum(h + 1, H - 1))
            sm = scores(b, q.astype(bf16), q[C:].astype(bf16))
            while todo and FIN[todo[0][0]] == b:
                finish(*todo.pop(0))
        if GP == 8:
            gate()
        if UP == 0:
            unpack_weights(jnp.minimum(h + 1, H - 1))
        q, v = project(0)
        q_s[...] = q.astype(bf16)
        todo.append(values(nb - 1, *sm))
        for t in todo:
            finish(*t)
        v_s[0:TQ, :] = v.astype(bf16)
        return carry

    if phases & 1:
        for cp in pair_copies(0, 0):
            cp.wait()
        unpack_weights(jnp.int32(0))
        q, v = project(0)
        q_s[...] = q.astype(bf16)
        v_s[0:TQ, :] = v.astype(bf16)
        if PEEL:
            head(jnp.int32(0), 0, WAITS[LATE])
        if phases == 3:
            for cp in tile_copies(0, 0):
                cp.start()
        lax.fori_loop(PEEL, H, head, 0, unroll=UNR)

    def mix(j, carry):
        slot = j & 1
        for cp in tile_copies(j, slot):
            cp.wait()

        @pl.when(j + 1 < NDT)
        def _():
            for cp in tile_copies(j + 1, 1 - slot):
                cp.start()

        @pl.when(j >= 2)
        def _():
            out_copy(j - 2, slot).wait()

        col = pl.ds(pl.multiple_of(j * C, C), C)
        zero = lax.shift_right_logical(j, 5)
        Z0, KV = H + zero, H + 2 + zero
        last = None
        prev = None
        for a in range(NC):
            hm = lax.dot_general(_ld(f_w, (), 0, 2 * C), pltpu.bitcast(ssm_w[slot, :, a * C:(a + 1) * C], bf16), NT, preferred_element_type=f32)
            ha = NC + a + zero
            if prev is None:
                sf_s[ha] = hm
            else:
                sf_s[ha, 0:64] = hm[0:64] - prev[128:192]
                sf_s[ha, 64:128] = hm[64:128] + prev[192:256]
                sf_s[ha, 128:192] = hm[128:192] + prev[0:64]
                sf_s[ha, 192:256] = hm[192:256] - prev[64:128]
            prev = hm
            if a == NC - 4:
                last = hm

        sk = sk_s[:, col].astype(f32)
        dd = d_s[...].astype(f32).reshape(NDT, C)
        dsel = jnp.sum(jnp.where(lax.broadcasted_iota(jnp.int32, (NDT, C), 0) == j, dd, 0.0), axis=0, keepdims=True)

        def short_steps():
            R = SR
            for n in range(S // R):
                if n == 0:
                    kk = jnp.concatenate([jnp.zeros((8, C), f32), _ld(akv_w, (slot, 0), 0, R).astype(f32)], axis=0)
                else:
                    kk = _ld(akv_w, (slot, 0), n * R - 16, R + 16).astype(f32)[8:]
                ks = kk[8:] * sk[0:1, :]
                for t in range(1, 4):
                    ks = ks + pltpu.roll(kk, t, 0)[8:] * sk[t:t + 1, :]
                rs = slice(n * R, (n + 1) * R)
                res_s[KV, rs] = (ks * _ld(akv_w, (slot, 1), n * R, R).astype(f32)).astype(bf16)
                yield

        done = [0]
        pending = []

        def branch_a(blk):
            for a in range(blk * NB, (blk + 1) * NB):
                rs = slice(a * C, (a + 1) * C)
                z = _ld(res_s, (Z0 + a // 8,), (a % 8) * 2 * C, 2 * C)
                y = _dot(_ld(g_w, (), 0, C), z) * (1.0 / C) + _ld(res_s, (KV,), a * C, C).astype(f32) * dsel
                av = gate_s[rs, :] * (pltpu.bitcast(x_w[a * C // 2:(a + 1) * C // 2, col], bf16).astype(f32) * y)
                if a * C // PR in pending:
                    o_b[slot, rs, :] = (av + b_s[rs, :]).astype(bf16)
                    if (a + 1) * C % PR == 0:
                        pending.remove(a * C // PR)
                else:
                    a_s[rs, :] = av
                done[0] = (a + 1) * C

        ready = []

        def conv_steps():
            for blk in range(NC // NB):
                outs = range(blk * NB, (blk + 1) * NB)
                for fr in range(C // 8):
                    re = slice(fr * 8, (fr + 1) * 8)
                    im = slice(C + fr * 8, C + (fr + 1) * 8)
                    hs = {}
                    z = {}
                    for b in range(outs[-1], -1, -1):
                        xr, xi = sf_s[b, re], sf_s[b, im]
                        for a in outs:
                            if a < b:
                                continue
                            if a - b not in hs:
                                hs[a - b] = (sf_s[NC + a - b, re], sf_s[NC + a - b, im])
                            hr, hi = hs[a - b]
                            tr = xr * hr - xi * hi
                            ti = xr * hi + xi * hr
                            z[a] = (tr, ti) if a not in z else (z[a][0] + tr, z[a][1] + ti)
                        if b == 0:
                            for a in outs:
                                res_s.bitcast(u32)[Z0 + a // 8, (a % 8) * C + fr * 8:(a % 8) * C + fr * 8 + 8] = (
                                    pltpu.pack_elementwise(list(z[a]), packed_dtype=bf16))
                            if fr == C // 8 - 1:
                                ready.append(blk)
                        yield

        NG = H // HG
        SL = PR // 32
        state = dict(prev=last, points=0, conv=0, short=0)
        sgen, cgen = short_steps(), conv_steps()
        nconv = (C // 8) * sum((blk + 1) * NB for blk in range(NC // NB))
        nshort = S // SR

        def proj(r):
            acc = None
            for g in range(NG):
                parts = []
                for i in range(SL):
                    rel = state["prev"][32 * i:32 * i + 8]
                    if r == 0:
                        want = min(nshort, -(-(g * SL + i + 1) * nshort // (NG * SL - SL)))
                        if want > state["short"]:
                            akv_w[slot + zero, 2, 0:8] = pltpu.bitcast(rel, u32)
                            while state["short"] < want:
                                next(sgen)
                                state["short"] += 1
                    else:
                        state["points"] += 1
                        want = min(nconv, -(-state["points"] * nconv // (NWIN * SL)))
                        if want > state["conv"]:
                            sf_s[2 * NC + zero, 0:8] = rel
                            while state["conv"] < want:
                                next(cgen)
                                state["conv"] += 1
                    parts.append(jnp.concatenate(
                        [_ld(res_s, (h,), r * PR + 32 * i, 32) for h in range(g * HG, (g + 1) * HG)], axis=1))
                t = _dot(jnp.concatenate(parts, axis=0), _ld(wo_w, (slot,), g * HG * DH, HG * DH))
                state["prev"] = t
                acc = t if acc is None else acc + t
                while ready:
                    branch_a(ready.pop(0))
            return acc

        for r in range(S // PR):
            acc = proj(r)
            if r == 0:
                for a in range(NC):
                    xm = _dot(_ld(f_w, (), 0, 2 * C), _ld(res_s, (KV,), a * C, C))
                    sf_s[a + zero] = xm
                state["prev"] = xm
            rs = slice(r * PR, (r + 1) * PR)
            if done[0] >= (r + 1) * PR:
                o_b[slot, rs, :] = (a_s[rs, :] + (1.0 - gate_s[rs, :]) * acc).astype(bf16)
            else:
                b_s[rs, :] = (1.0 - gate_s[rs, :]) * acc
                pending.append(r)
        assert not pending and state["conv"] == nconv and state["short"] == nshort
        out_copy(j, slot).start()
        return carry

    if phases & 2:
        lax.fori_loop(0, NDT, mix, 0)
        out_copy(NDT - 2, 0).wait()
        out_copy(NDT - 1, 1).wait()


def make(phases=3):
    @jax.jit
    def fn(A_q, A_k, A_v, A_shift_k, A_ssm_k, A_ssm_D, B_x, B_c_kv, B_w_q, B_w_uk, B_w_uv, B_w_o, gate_w):
        fwd, inv = _dft_matrices()
        V = pltpu.VMEM
        out = pl.pallas_call(
            functools.partial(_kernel, phases=phases),
            in_specs=[pl.BlockSpec(memory_space=pl.ANY)] * 14,
            out_specs=pl.BlockSpec(memory_space=pl.ANY),
            out_shape=jax.ShapeDtypeStruct((S, M), bf16),
            scratch_shapes=[
                V((S // 2, M), u32), V((S // 2, DC), u32),
                V((2, M, DH), u32), V((2, DC, DH), u32), V((2, DC, DH), u32),
                V((2, H * DH // 2, C), u32), V((2, 3, S // 2, C), u32), V((2, C // 2, S), u32),
                V((2, S, C), bf16),
                V((4, M), bf16), V((M,), bf16), V((M,), bf16), V((C, C), u32), V((C // 2, 2 * C), u32),
                V((TQ, DH), bf16), V((TQ, DH), bf16),
                V((NC, DH, C), bf16), V((S, DH), bf16),
                V((H + 4, S, DH), bf16), V((S, C), f32),
                V((2 * NC + 1, 2 * C, C), f32), V((S, C), f32), V((S, C), f32),
                pltpu.SemaphoreType.DMA((5,)), pltpu.SemaphoreType.DMA((2, S // TQ)),
                pltpu.SemaphoreType.DMA((3, 2)), pltpu.SemaphoreType.DMA((4, 2)), pltpu.SemaphoreType.DMA((2,)),
            ],
            compiler_params=pltpu.CompilerParams(vmem_limit_bytes=100 * 1024 * 1024),
            name="fused",
        )(A_q.reshape(S, M), B_c_kv.reshape(S, DC), B_w_q, B_w_uk, B_w_uv, B_w_o.reshape(H * DH, M),
          A_k.reshape(S, M), A_v.reshape(S, M), A_shift_k.T, A_ssm_k, A_ssm_D, gate_w,
          fwd.astype(bf16), inv.astype(bf16))
        return out.reshape(1, S, M)
    return fn


pallas_gated_mix__ssm_conv_h3__compressed_kv_cla__prompt_kernel = make(3)
```

```python
import functools

import jax
import jax.numpy as jnp
import numpy as np
from jax import lax
from jax.experimental import pallas as pl
from jax.experimental.pallas import tpu as pltpu

S = 2048
H = 32
DH = 128
M = 1024
DC = 512
C = 128
NC = S // C
NDT = M // C
TQ = 256
NB = 4
HG = 4
SR = 32
NWIN = 52
Z_SLAB = H
KV_SLAB = H + 4
W_SLAB = H + 5
FIRST_HEAD_WAITS = {1: (1,), 2: (2,), 3: (3,), 4: (4, 5), 6: (6, 7)}

MASKED = -999292928.0
NEG = -1e30
LOG2E = 1.4426950408889634
NT = (((1,), (1,)), ((), ()))
f32 = jnp.float32
bf16 = jnp.bfloat16
u32 = jnp.uint32


def _dft_matrices():
    k = np.concatenate([np.arange(0, C, 2), np.arange(1, C, 2)]).astype(np.float64)
    t = np.arange(C, dtype=np.float64)
    th = 2.0 * np.pi * (k[:, None] + 0.5) * t[None, :] / (2 * C)
    fwd = np.concatenate([np.cos(th), -np.sin(th)], axis=0)
    return fwd, np.ascontiguousarray(fwd.T)


def _dot(a, b):
    return jnp.dot(a, b, preferred_element_type=f32)


def _ld(ref, lead, r0, n):
    w = ref if ref.dtype == u32 else ref.bitcast(u32)
    start = r0 // 2 if isinstance(r0, int) else r0
    return pltpu.bitcast(w[(*lead, pl.ds(start, n // 2), slice(None))], bf16)


def _recip(l):
    r = pl.reciprocal(l, approx=True)
    return r * (2.0 - l * r)


def _kernel(x_hbm, c_hbm, wq_hbm, wuk_hbm, wuv_hbm, wo_hbm, ak_hbm, av_hbm, sk_hbm, ssm_hbm,
            d_hbm, gw_hbm, f_hbm, g_hbm, o_hbm,
            x_w, c_w, wq_b, wk_b, wv_b, wo_w, akv_w, ssm_w, o_b, sk_s, d_s, gw_s, f_w, g_w,
            q_s, k_s, kt_s, v_s, res_s, gate_s, low_s, sf_s, a_s, b_s,
            sem_in, sem_r, sem_w, sem_t, sem_o):

    def pair_copies(p, slot):
        return [pltpu.make_async_copy(w.bitcast(u32).at[:, p], b.at[slot], sem_w.at[n, slot])
                for n, (w, b) in enumerate(((wuk_hbm, wk_b), (wuv_hbm, wv_b), (wq_hbm, wq_b)))]

    def tile_copies(j, slot):
        col = pl.ds(pl.multiple_of(j * C, C), C)
        row = pl.ds(pl.multiple_of(j * (C // 2), C // 2), C // 2)
        return [pltpu.make_async_copy(src, dst, sem_t.at[n, slot])
                for n, (src, dst) in enumerate((
                    (ssm_hbm.bitcast(u32).at[row, :], ssm_w.at[slot]),
                    (ak_hbm.bitcast(u32).at[:, col], akv_w.at[slot, 0]),
                    (av_hbm.bitcast(u32).at[:, col], akv_w.at[slot, 1]),
                    (wo_hbm.bitcast(u32).at[:, col], wo_w.at[slot])))]

    def out_copy(j, slot):
        col = pl.ds(pl.multiple_of(j * C, C), C)
        return pltpu.make_async_copy(o_b.at[slot], o_hbm.at[:, col], sem_o.at[slot])

    row_cp = [[pltpu.make_async_copy(src.bitcast(u32).at[b * TQ // 2:(b + 1) * TQ // 2, :],
                                     dst.at[b * TQ // 2:(b + 1) * TQ // 2, :], sem_r.at[n, b])
               for n, (src, dst) in enumerate(((c_hbm, c_w), (x_hbm, x_w)))]
              for b in range(S // TQ)]
    small = [pltpu.make_async_copy(s, d, sem_in.at[n]) for n, (s, d) in enumerate((
        (gw_hbm, gw_s), (sk_hbm, sk_s), (d_hbm, d_s),
        (f_hbm.bitcast(u32), f_w), (g_hbm.bitcast(u32), g_w)))]
    for cp in pair_copies(0, 0) + row_cp[0] + small + sum(row_cp[1:], []):
        cp.start()
    for cp in row_cp[0] + small:
        cp.wait()

    def unpack_weights(h):
        slot = lax.shift_right_logical(h, 1) & 1
        sh = ((h & 1) * 16).astype(u32)
        for b, n0, n in ((wk_b, 0, DC), (wv_b, DC, DC), (wq_b, 2 * DC, M)):
            w = lax.shift_left(b[slot], 16 - sh) & np.uint32(0xFFFF0000)
            res_s[W_SLAB, n0:n0 + n, :] = pltpu.bitcast(w, f32).astype(bf16)

    def project(b):
        kv = _dot(_ld(c_w, (), b * TQ, TQ),
                  jnp.concatenate([_ld(res_s, (W_SLAB,), 0, DC), _ld(res_s, (W_SLAB,), DC, DC)], axis=1))
        k_s[...] = kv[:, :DH].astype(bf16)
        for t in range(TQ // C):
            kt_s[b * TQ // C + t] = _ld(k_s, (), t * C, C).T
        q = _dot(_ld(x_w, (), b * TQ, TQ), _ld(res_s, (W_SLAB,), 2 * DC, M)) * (DH ** -0.5 * LOG2E)
        return q, kv[:, DH:]

    def head(h, carry, waits=None):
        p = lax.shift_right_logical(h, 1) + 1

        @pl.when(((h & 1) == 0) & (p < H // 2))
        def _():
            for cp in pair_copies(p, p & 1):
                cp.start()

        @pl.when(((h & 1) == 1) & (p < H // 2))
        def _():
            for cp in pair_copies(p, p & 1):
                cp.wait()

        tri = lax.broadcasted_iota(jnp.int32, (C, C), 1) <= lax.broadcasted_iota(jnp.int32, (C, C), 0)

        def scores(b, q, q2):
            r0 = b * TQ
            s1 = _dot(q, jnp.concatenate([_ld(kt_s, (t,), 0, C) for t in range(2 * b + 1)], axis=1))
            s2 = jnp.where(tri, _dot(q2, _ld(kt_s, (2 * b + 1,), 0, C)), NEG)
            diag = jnp.concatenate([jnp.where(tri, s1[:C, r0:], NEG), s1[C:, r0:]], axis=0)
            tiles = [s1[:, t * C:(t + 1) * C] for t in range(2 * b)] + [diag]
            m = functools.reduce(jnp.maximum, tiles)
            m = jnp.concatenate([m[:C], jnp.maximum(m[C:], s2)], axis=0)
            m = jnp.broadcast_to(jnp.max(m, axis=-1, keepdims=True), (TQ, C))
            lows.append(jnp.min(m.reshape(TQ // 8, 8, C), axis=0))
            return tiles, s2, m

        def values(b, tiles, s2, m):
            n1 = b * TQ + C
            ps = [jnp.exp2(t - m) for t in tiles]
            p2 = jnp.exp2(s2 - m[C:])
            o = _dot(jnp.concatenate(ps, axis=1).astype(bf16), _ld(v_s, (), 0, n1))
            ob = o[C:] + _dot(p2.astype(bf16), _ld(v_s, (), n1, C))
            l = functools.reduce(jnp.add, ps)
            l = jnp.concatenate([l[:C], l[C:] + p2], axis=0)
            return b, jnp.concatenate([o[:C], ob], axis=0), l

        def finish(b, o, l):
            l = _recip(jnp.broadcast_to(jnp.sum(l, axis=-1, keepdims=True), (TQ, DH)))
            res_s[h, b * TQ:(b + 1) * TQ, :] = (o * l).astype(bf16)

        nb = S // TQ
        todo = []
        lows = [low_s[...]]
        sm = scores(0, _ld(q_s, (), 0, TQ), _ld(q_s, (), C, C))
        for b in range(1, nb):
            for n in (waits or {}).get(b, ()):
                for cp in row_cp[n]:
                    cp.wait()
            q, v = project(b)
            v_s[b * TQ:(b + 1) * TQ, :] = v.astype(bf16)
            todo.append(values(b - 1, *sm))
            sm = scores(b, q.astype(bf16), q[C:].astype(bf16))

        gr = S // H
        xg = pltpu.bitcast(x_w[pl.ds(pl.multiple_of(h * (gr // 2), gr // 2), gr // 2), :], bf16)
        gl = jnp.sum(xg.astype(f32) * gw_s[...].astype(f32).reshape(1, M), axis=-1, keepdims=True)
        gate_s[pl.ds(pl.multiple_of(h * gr, gr), gr), :] = jax.nn.sigmoid(jnp.broadcast_to(gl, (gr, C)))

        unpack_weights(jnp.minimum(h + 1, H - 1))
        q, v = project(0)
        q_s[...] = q.astype(bf16)
        todo.append(values(nb - 1, *sm))
        for t in todo:
            finish(*t)
        v_s[0:TQ, :] = v.astype(bf16)
        low_s[...] = functools.reduce(jnp.minimum, lows)
        return carry

    def unskipped_head(h, carry):
        p = lax.shift_right_logical(h, 1)
        for cp in pair_copies(p, p & 1):
            cp.start()
        for cp in pair_copies(p, p & 1):
            cp.wait()
        unpack_weights(h)

        def proj(t, carry):
            w0 = pl.multiple_of(t * (C // 2), C // 2)
            rows = pl.ds(pl.multiple_of(t * C, C), C)
            cb = _ld(c_w, (), w0, C)
            k_s[0:C] = _dot(cb, _ld(res_s, (W_SLAB,), 0, DC)).astype(bf16)
            kt_s[t] = _ld(k_s, (), 0, C).T
            v_s[rows, :] = _dot(cb, _ld(res_s, (W_SLAB,), DC, DC)).astype(bf16)
            a_s[rows, :] = _dot(_ld(x_w, (), w0, C), _ld(res_s, (W_SLAB,), 2 * DC, M)) * (DH ** -0.5 * LOG2E)
            return carry

        def attend(t, carry):
            rows = pl.ds(pl.multiple_of(t * C, C), C)
            s = _dot(a_s[rows, :].astype(bf16),
                     jnp.concatenate([_ld(kt_s, (n,), 0, C) for n in range(NC)], axis=1))
            keep = (lax.broadcasted_iota(jnp.int32, (C, S), 1)
                    <= t * C + lax.broadcasted_iota(jnp.int32, (C, S), 0))
            s = jnp.where(keep, s, MASKED * LOG2E)
            e = jnp.exp2(s - jnp.max(s, axis=-1, keepdims=True))
            o = _dot(e.astype(bf16), _ld(v_s, (), 0, S)) / jnp.sum(e, axis=-1, keepdims=True)
            res_s[h, rows, :] = o.astype(bf16)
            return carry

        lax.fori_loop(0, NC, proj, 0)
        lax.fori_loop(0, NC, attend, 0)
        return carry

    low_s[...] = jnp.zeros(low_s.shape, f32)
    for cp in pair_copies(0, 0):
        cp.wait()
    first = jnp.zeros((), jnp.int32)
    unpack_weights(first)
    q, v = project(0)
    q_s[...] = q.astype(bf16)
    v_s[0:TQ, :] = v.astype(bf16)
    head(first, 0, FIRST_HEAD_WAITS)
    for cp in tile_copies(0, 0):
        cp.start()
    lax.fori_loop(1, H, head, 0)

    @pl.when(jnp.min(low_s[...]) < 0.99 * MASKED * LOG2E)
    def _():
        lax.fori_loop(0, H, unskipped_head, 0)

    def mix(j, carry):
        slot = j & 1
        for cp in tile_copies(j, slot):
            cp.wait()

        @pl.when(j + 1 < NDT)
        def _():
            for cp in tile_copies(j + 1, 1 - slot):
                cp.start()

        @pl.when(j >= 2)
        def _():
            out_copy(j - 2, slot).wait()

        col = pl.ds(pl.multiple_of(j * C, C), C)
        zero = lax.shift_right_logical(j, 5)
        Z0, KV = Z_SLAB + zero, KV_SLAB + zero

        last = prev = None
        for a in range(NC):
            hm = lax.dot_general(_ld(f_w, (), 0, 2 * C),
                                 pltpu.bitcast(ssm_w[slot, :, a * C:(a + 1) * C], bf16),
                                 NT, preferred_element_type=f32)
            ha = NC + a + zero
            if prev is None:
                sf_s[ha] = hm
            else:
                sf_s[ha, 0:64] = hm[0:64] - prev[128:192]
                sf_s[ha, 64:128] = hm[64:128] + prev[192:256]
                sf_s[ha, 128:192] = hm[128:192] + prev[0:64]
                sf_s[ha, 192:256] = hm[192:256] - prev[64:128]
            prev = hm
            if a == NC - 4:
                last = hm

        sk = sk_s[:, col].astype(f32)
        dd = d_s[...].astype(f32).reshape(NDT, C)
        dsel = jnp.sum(jnp.where(lax.broadcasted_iota(jnp.int32, (NDT, C), 0) == j, dd, 0.0),
                       axis=0, keepdims=True)

        def short_steps():
            for n in range(S // SR):
                if n == 0:
                    kk = jnp.concatenate(
                        [jnp.zeros((8, C), f32), _ld(akv_w, (slot, 0), 0, SR).astype(f32)], axis=0)
                else:
                    kk = _ld(akv_w, (slot, 0), n * SR - 16, SR + 16).astype(f32)[8:]
                ks = kk[8:] * sk[0:1, :]
                for t in range(1, 4):
                    ks = ks + pltpu.roll(kk, t, 0)[8:] * sk[t:t + 1, :]
                res_s[KV, n * SR:(n + 1) * SR] = (
                    ks * _ld(akv_w, (slot, 1), n * SR, SR).astype(f32)).astype(bf16)
                yield

        ready = []

        def conv_steps():
            for blk in range(NC // NB):
                outs = range(blk * NB, (blk + 1) * NB)
                for fr in range(C // 8):
                    re = slice(fr * 8, (fr + 1) * 8)
                    im = slice(C + fr * 8, C + (fr + 1) * 8)
                    hs = {}
                    z = {}
                    for b in range(outs[-1], -1, -1):
                        xr, xi = sf_s[b, re], sf_s[b, im]
                        for a in outs:
                            if a < b:
                                continue
                            if a - b not in hs:
                                hs[a - b] = (sf_s[NC + a - b, re], sf_s[NC + a - b, im])
                            hr, hi = hs[a - b]
                            tr = xr * hr - xi * hi
                            ti = xr * hi + xi * hr
                            z[a] = (tr, ti) if a not in z else (z[a][0] + tr, z[a][1] + ti)
                        if b == 0:
                            for a in outs:
                                for part, z0 in zip(z[a], (0, C)):
                                    z0 += (a % 4) * 2 * C + fr * 8
                                    res_s.bitcast(u32)[Z0 + a // 4, z0:z0 + 8] = pltpu.bitcast(part, u32)
                            if fr == C // 8 - 1:
                                ready.append(blk)
                        yield

        done = [0]
        pending = []

        def branch_a(blk):
            for a in range(blk * NB, (blk + 1) * NB):
                rs = slice(a * C, (a + 1) * C)
                z = res_s.bitcast(u32)[Z0 + a // 4, (a % 4) * 2 * C:(a % 4 + 1) * 2 * C]
                y = (_dot(_ld(g_w, (), 0, C), pltpu.bitcast(z, f32).astype(bf16)) * (1.0 / C)
                     + _ld(res_s, (KV,), a * C, C).astype(f32) * dsel)
                xq = pltpu.bitcast(x_w[a * C // 2:(a + 1) * C // 2, col], bf16).astype(f32)
                av = gate_s[rs, :] * (xq * y)
                if a * C // TQ in pending:
                    o_b[slot, rs, :] = (av + b_s[rs, :]).astype(bf16)
                    if (a + 1) * C % TQ == 0:
                        pending.remove(a * C // TQ)
                else:
                    a_s[rs, :] = av
                done[0] = (a + 1) * C

        NG = H // HG
        SL = TQ // 32
        state = dict(prev=last, points=0, conv=0, short=0)
        sgen, cgen = short_steps(), conv_steps()
        nconv = (C // 8) * sum((blk + 1) * NB for blk in range(NC // NB))
        nshort = S // SR

        def out_proj(r):
            acc = None
            for g in range(NG):
                parts = []
                for i in range(SL):
                    mark = state["prev"][32 * i:32 * i + 8]
                    if r == 0:
                        want = min(nshort, -(-(g * SL + i + 1) * nshort // ((NG - 1) * SL)))
                        if want > state["short"]:
                            akv_w[slot + zero, 2, 0:8] = pltpu.bitcast(mark, u32)
                            while state["short"] < want:
                                next(sgen)
                                state["short"] += 1
                    elif r > 1 or g >= 1:
                        state["points"] += 1
                        want = min(nconv, -(-state["points"] * nconv // (NWIN * SL)))
                        if want > state["conv"]:
                            sf_s[2 * NC + zero, 0:8] = mark
                            while state["conv"] < want:
                                next(cgen)
                                state["conv"] += 1
                    parts.append(jnp.concatenate(
                        [_ld(res_s, (h,), r * TQ + 32 * i, 32) for h in range(g * HG, (g + 1) * HG)], axis=1))
                t = _dot(jnp.concatenate(parts, axis=0), _ld(wo_w, (slot,), g * HG * DH, HG * DH))
                state["prev"] = t
                acc = t if acc is None else acc + t
                while ready:
                    branch_a(ready.pop(0))
            return acc

        for r in range(S // TQ):
            acc = out_proj(r)
            if r == 0:
                for a in range(NC):
                    xm = _dot(_ld(f_w, (), 0, 2 * C), _ld(res_s, (KV,), a * C, C))
                    sf_s[a + zero] = xm
                state["prev"] = xm
            rs = slice(r * TQ, (r + 1) * TQ)
            if done[0] >= (r + 1) * TQ:
                o_b[slot, rs, :] = (a_s[rs, :] + (1.0 - gate_s[rs, :]) * acc).astype(bf16)
            else:
                b_s[rs, :] = (1.0 - gate_s[rs, :]) * acc
                pending.append(r)
        assert not pending and state["conv"] == nconv and state["short"] == nshort
        out_copy(j, slot).start()
        return carry

    lax.fori_loop(0, NDT, mix, 0)
    out_copy(NDT - 2, 0).wait()
    out_copy(NDT - 1, 1).wait()


@jax.jit
def pallas_gated_mix__ssm_conv_h3__compressed_kv_cla__prompt_kernel(
    A_q: jax.Array,
    A_k: jax.Array,
    A_v: jax.Array,
    A_shift_k: jax.Array,
    A_ssm_k: jax.Array,
    A_ssm_D: jax.Array,
    B_x: jax.Array,
    B_c_kv: jax.Array,
    B_w_q: jax.Array,
    B_w_uk: jax.Array,
    B_w_uv: jax.Array,
    B_w_o: jax.Array,
    gate_w: jax.Array,
):
    del B_x
    fwd, inv = _dft_matrices()
    V = pltpu.VMEM
    dma = pltpu.SemaphoreType.DMA
    out = pl.pallas_call(
        _kernel,
        in_specs=[pl.BlockSpec(memory_space=pl.ANY)] * 14,
        out_specs=pl.BlockSpec(memory_space=pl.ANY),
        out_shape=jax.ShapeDtypeStruct((S, M), bf16),
        scratch_shapes=[
            V((S // 2, M), u32), V((S // 2, DC), u32),
            V((2, M, DH), u32), V((2, DC, DH), u32), V((2, DC, DH), u32),
            V((2, H * DH // 2, C), u32), V((2, 3, S // 2, C), u32),
            V((2, C // 2, S), u32), V((2, S, C), bf16),
            V((4, M), bf16), V((M,), bf16), V((M,), bf16),
            V((C, C), u32), V((C // 2, 2 * C), u32),
            V((TQ, DH), bf16), V((TQ, DH), bf16), V((NC, DH, C), bf16), V((S, DH), bf16),
            V((H + 6, S, DH), bf16), V((S, C), f32), V((8, C), f32),
            V((2 * NC + 1, 2 * C, C), f32), V((S, C), f32), V((S, C), f32),
            dma((5,)), dma((2, S // TQ)), dma((3, 2)), dma((4, 2)), dma((2,)),
        ],
        compiler_params=pltpu.CompilerParams(vmem_limit_bytes=100 * 1024 * 1024),
        name="fused",
    )(A_q.reshape(S, M), B_c_kv.reshape(S, DC), B_w_q, B_w_uk, B_w_uv, B_w_o.reshape(H * DH, M),
      A_k.reshape(S, M), A_v.reshape(S, M), A_shift_k.T, A_ssm_k, A_ssm_D, gate_w,
      fwd.astype(bf16), inv.astype(bf16))
    return out.reshape(1, S, M)
```

```python
import functools

import jax
import jax.numpy as jnp
import numpy as np
from jax import lax
from jax.experimental import pallas as pl
from jax.experimental.pallas import tpu as pltpu

S = 2048
H = 32
DH = 128
M = 1024
DC = 512
C = 128
NC = S // C
NDT = M // C
TQ = 256
NB = 4
HG = 4
SR = 32
NWIN = 44
Z_SLAB = H
KV_SLAB = H + 4
W_SLAB = H + 5
FIRST_HEAD_WAITS = {1: (1,), 2: (2,), 3: (3,), 4: (4, 5), 6: (6, 7)}

MASKED = -999292928.0
NEG = -1e30
LOG2E = 1.4426950408889634
NT = (((1,), (1,)), ((), ()))
f32 = jnp.float32
bf16 = jnp.bfloat16
u32 = jnp.uint32


def _dft_matrices():
    even = np.arange(0, C, 2)
    k = np.concatenate([even, C - 1 - even]).astype(np.float64)
    th = 2.0 * np.pi * (k[:, None] + 0.5) * np.arange(C, dtype=np.float64)[None, :] / (2 * C)
    fwd = np.concatenate([np.cos(th), -np.sin(th)], axis=0)
    half = np.concatenate([np.cos(th[:C // 2]), -np.sin(th[:C // 2])], axis=0).T
    return fwd, np.concatenate([half[0::2], half[1::2]], axis=0)


def _dot(a, b):
    return jnp.dot(a, b, preferred_element_type=f32)


def _ld(ref, lead, r0, n):
    w = ref if ref.dtype == u32 else ref.bitcast(u32)
    start = r0 // 2 if isinstance(r0, int) else r0
    return pltpu.bitcast(w[(*lead, pl.ds(start, n // 2), slice(None))], bf16)


def _recip(l):
    r = pl.reciprocal(l, approx=True)
    return r * (2.0 - l * r)


def _kernel(x_hbm, c_hbm, wq_hbm, wuk_hbm, wuv_hbm, wo_hbm, ak_hbm, av_hbm, sk_hbm, ssm_hbm,
            d_hbm, gw_hbm, f_hbm, g_hbm, o_hbm,
            x_w, c_w, wq_b, wk_b, wv_b, wo_w, akv_w, ssm_w, o_b, sk_s, d_s, gw_s, f_w, g_w,
            q_s, k_s, kt_s, v_s, res_s, gate_s, low_s, sf_s, a_s, b_s,
            sem_in, sem_r, sem_w, sem_t, sem_o):

    def pair_copies(p, slot):
        return [pltpu.make_async_copy(w.bitcast(u32).at[:, p], b.at[slot], sem_w.at[n, slot])
                for n, (w, b) in enumerate(((wuk_hbm, wk_b), (wuv_hbm, wv_b), (wq_hbm, wq_b)))]

    def tile_copies(j, slot):
        col = pl.ds(pl.multiple_of(j * C, C), C)
        row = pl.ds(pl.multiple_of(j * (C // 2), C // 2), C // 2)
        return [pltpu.make_async_copy(src, dst, sem_t.at[n, slot])
                for n, (src, dst) in enumerate((
                    (ssm_hbm.bitcast(u32).at[row, :], ssm_w.at[slot]),
                    (ak_hbm.bitcast(u32).at[:, col], akv_w.at[slot, 0]),
                    (av_hbm.bitcast(u32).at[:, col], akv_w.at[slot, 1]),
                    (wo_hbm.bitcast(u32).at[:, col], wo_w.at[slot])))]

    def out_copy(j, slot):
        col = pl.ds(pl.multiple_of(j * C, C), C)
        return pltpu.make_async_copy(o_b.at[slot], o_hbm.at[:, col], sem_o.at[slot])

    row_cp = [[pltpu.make_async_copy(src.bitcast(u32).at[b * TQ // 2:(b + 1) * TQ // 2, :],
                                     dst.at[b * TQ // 2:(b + 1) * TQ // 2, :], sem_r.at[n, b])
               for n, (src, dst) in enumerate(((c_hbm, c_w), (x_hbm, x_w)))]
              for b in range(S // TQ)]
    small = [pltpu.make_async_copy(s, d, sem_in.at[n]) for n, (s, d) in enumerate((
        (gw_hbm, gw_s), (sk_hbm, sk_s), (d_hbm, d_s),
        (f_hbm.bitcast(u32), f_w), (g_hbm.bitcast(u32), g_w)))]
    for cp in pair_copies(0, 0) + row_cp[0] + small + sum(row_cp[1:], []):
        cp.start()
    for cp in row_cp[0] + small:
        cp.wait()

    def unpack_weights(h):
        slot = lax.shift_right_logical(h, 1) & 1
        sh = ((h & 1) * 16).astype(u32)
        for b, n0, n in ((wk_b, 0, DC), (wv_b, DC, DC), (wq_b, 2 * DC, M)):
            w = lax.shift_left(b[slot], 16 - sh) & np.uint32(0xFFFF0000)
            res_s[W_SLAB, n0:n0 + n, :] = pltpu.bitcast(w, f32).astype(bf16)

    def project(b):
        kv = _dot(_ld(c_w, (), b * TQ, TQ),
                  jnp.concatenate([_ld(res_s, (W_SLAB,), 0, DC), _ld(res_s, (W_SLAB,), DC, DC)], axis=1))
        k_s[...] = kv[:, :DH].astype(bf16)
        for t in range(TQ // C):
            kt_s[b * TQ // C + t] = _ld(k_s, (), t * C, C).T
        q = _dot(_ld(x_w, (), b * TQ, TQ), _ld(res_s, (W_SLAB,), 2 * DC, M)) * (DH ** -0.5 * LOG2E)
        return q, kv[:, DH:]

    def head(h, carry, waits=None):
        p = lax.shift_right_logical(h, 1) + 1

        @pl.when(((h & 1) == 0) & (p < H // 2))
        def _():
            for cp in pair_copies(p, p & 1):
                cp.start()

        @pl.when(((h & 1) == 1) & (p < H // 2))
        def _():
            for cp in pair_copies(p, p & 1):
                cp.wait()

        tri = lax.broadcasted_iota(jnp.int32, (C, C), 1) <= lax.broadcasted_iota(jnp.int32, (C, C), 0)

        def scores(b, q, q2):
            r0 = b * TQ
            s1 = _dot(q, jnp.concatenate([_ld(kt_s, (t,), 0, C) for t in range(2 * b + 1)], axis=1))
            s2 = jnp.where(tri, _dot(q2, _ld(kt_s, (2 * b + 1,), 0, C)), NEG)
            diag = jnp.concatenate([jnp.where(tri, s1[:C, r0:], NEG), s1[C:, r0:]], axis=0)
            tiles = [s1[:, t * C:(t + 1) * C] for t in range(2 * b)] + [diag]
            m = functools.reduce(jnp.maximum, tiles)
            m = jnp.concatenate([m[:C], jnp.maximum(m[C:], s2)], axis=0)
            m = jnp.broadcast_to(jnp.max(m, axis=-1, keepdims=True), (TQ, C))
            lows.append(jnp.min(m.reshape(TQ // 8, 8, C), axis=0))
            return tiles, s2, m

        def values(b, tiles, s2, m):
            n1 = b * TQ + C
            ps = [jnp.exp2(t - m) for t in tiles]
            p2 = jnp.exp2(s2 - m[C:])
            o = _dot(jnp.concatenate(ps, axis=1).astype(bf16), _ld(v_s, (), 0, n1))
            ob = o[C:] + _dot(p2.astype(bf16), _ld(v_s, (), n1, C))
            l = functools.reduce(jnp.add, ps)
            l = jnp.concatenate([l[:C], l[C:] + p2], axis=0)
            return b, jnp.concatenate([o[:C], ob], axis=0), l

        def finish(b, o, l):
            l = _recip(jnp.broadcast_to(jnp.sum(l, axis=-1, keepdims=True), (TQ, DH)))
            res_s[h, b * TQ:(b + 1) * TQ, :] = (o * l).astype(bf16)

        nb = S // TQ
        todo = []
        lows = [low_s[...]]
        sm = scores(0, _ld(q_s, (), 0, TQ), _ld(q_s, (), C, C))
        for b in range(1, nb):
            for n in (waits or {}).get(b, ()):
                for cp in row_cp[n]:
                    cp.wait()
            q, v = project(b)
            v_s[b * TQ:(b + 1) * TQ, :] = v.astype(bf16)
            todo.append(values(b - 1, *sm))
            sm = scores(b, q.astype(bf16), q[C:].astype(bf16))

        gr = S // H
        xg = pltpu.bitcast(x_w[pl.ds(pl.multiple_of(h * (gr // 2), gr // 2), gr // 2), :], bf16)
        gl = jnp.sum(xg.astype(f32) * gw_s[...].astype(f32).reshape(1, M), axis=-1, keepdims=True)
        gate_s[pl.ds(pl.multiple_of(h * gr, gr), gr), :] = jax.nn.sigmoid(jnp.broadcast_to(gl, (gr, C)))

        unpack_weights(jnp.minimum(h + 1, H - 1))
        q, v = project(0)
        q_s[...] = q.astype(bf16)
        todo.append(values(nb - 1, *sm))
        for t in todo:
            finish(*t)
        v_s[0:TQ, :] = v.astype(bf16)
        low_s[...] = functools.reduce(jnp.minimum, lows)
        return carry

    def unskipped_head(h, carry):
        p = lax.shift_right_logical(h, 1)
        for cp in pair_copies(p, p & 1):
            cp.start()
        for cp in pair_copies(p, p & 1):
            cp.wait()
        unpack_weights(h)

        def proj(t, carry):
            w0 = pl.multiple_of(t * (C // 2), C // 2)
            rows = pl.ds(pl.multiple_of(t * C, C), C)
            cb = _ld(c_w, (), w0, C)
            k_s[0:C] = _dot(cb, _ld(res_s, (W_SLAB,), 0, DC)).astype(bf16)
            kt_s[t] = _ld(k_s, (), 0, C).T
            v_s[rows, :] = _dot(cb, _ld(res_s, (W_SLAB,), DC, DC)).astype(bf16)
            a_s[rows, :] = _dot(_ld(x_w, (), w0, C), _ld(res_s, (W_SLAB,), 2 * DC, M)) * (DH ** -0.5 * LOG2E)
            return carry

        def attend(t, carry):
            rows = pl.ds(pl.multiple_of(t * C, C), C)
            s = _dot(a_s[rows, :].astype(bf16),
                     jnp.concatenate([_ld(kt_s, (n,), 0, C) for n in range(NC)], axis=1))
            keep = (lax.broadcasted_iota(jnp.int32, (C, S), 1)
                    <= t * C + lax.broadcasted_iota(jnp.int32, (C, S), 0))
            s = jnp.where(keep, s, MASKED * LOG2E)
            e = jnp.exp2(s - jnp.max(s, axis=-1, keepdims=True))
            o = _dot(e.astype(bf16), _ld(v_s, (), 0, S)) / jnp.sum(e, axis=-1, keepdims=True)
            res_s[h, rows, :] = o.astype(bf16)
            return carry

        lax.fori_loop(0, NC, proj, 0)
        lax.fori_loop(0, NC, attend, 0)
        return carry

    low_s[...] = jnp.zeros(low_s.shape, f32)
    for cp in pair_copies(0, 0):
        cp.wait()
    first = jnp.zeros((), jnp.int32)
    unpack_weights(first)
    q, v = project(0)
    q_s[...] = q.astype(bf16)
    v_s[0:TQ, :] = v.astype(bf16)
    head(first, 0, FIRST_HEAD_WAITS)
    for cp in tile_copies(0, 0):
        cp.start()
    lax.fori_loop(1, H, head, 0)

    @pl.when(jnp.min(low_s[...]) < 0.99 * MASKED * LOG2E)
    def _():
        lax.fori_loop(0, H, unskipped_head, 0)

    def mix(j, carry):
        slot = j & 1
        for cp in tile_copies(j, slot):
            cp.wait()

        @pl.when(j + 1 < NDT)
        def _():
            for cp in tile_copies(j + 1, 1 - slot):
                cp.start()

        @pl.when(j >= 2)
        def _():
            out_copy(j - 2, slot).wait()

        col = pl.ds(pl.multiple_of(j * C, C), C)
        zero = lax.shift_right_logical(j, 5)
        Z0, KV = Z_SLAB + zero, KV_SLAB + zero

        last = prev = None
        for a in range(NC):
            hm = lax.dot_general(_ld(f_w, (), 0, 2 * C),
                                 pltpu.bitcast(ssm_w[slot, :, a * C:(a + 1) * C], bf16),
                                 NT, preferred_element_type=f32)
            ha = NC + a + zero
            if prev is None:
                sf_s[ha] = hm
            else:
                sf_s[ha, 0:64] = hm[0:64] - prev[128:192]
                sf_s[ha, 64:128] = hm[64:128] + prev[192:256]
                sf_s[ha, 128:192] = hm[128:192] + prev[0:64]
                sf_s[ha, 192:256] = hm[192:256] - prev[64:128]
            prev = hm
            if a == NC - 4:
                last = hm

        sk = sk_s[:, col].astype(f32)
        dd = d_s[...].astype(f32).reshape(NDT, C)
        dsel = jnp.sum(jnp.where(lax.broadcasted_iota(jnp.int32, (NDT, C), 0) == j, dd, 0.0),
                       axis=0, keepdims=True)

        def short_steps():
            for n in range(S // SR):
                if n == 0:
                    kk = jnp.concatenate(
                        [jnp.zeros((8, C), f32), _ld(akv_w, (slot, 0), 0, SR).astype(f32)], axis=0)
                else:
                    kk = _ld(akv_w, (slot, 0), n * SR - 16, SR + 16).astype(f32)[8:]
                ks = kk[8:] * sk[0:1, :]
                for t in range(1, 4):
                    ks = ks + pltpu.roll(kk, t, 0)[8:] * sk[t:t + 1, :]
                res_s[KV, n * SR:(n + 1) * SR] = (
                    ks * _ld(akv_w, (slot, 1), n * SR, SR).astype(f32)).astype(bf16)
                yield

        ready, settled = [], []

        def conv_steps():
            for blk in range(NC // NB):
                outs = range(blk * NB, (blk + 1) * NB)
                for fr in range(C // 8):
                    re = slice(fr * 8, (fr + 1) * 8)
                    im = slice(C + fr * 8, C + (fr + 1) * 8)
                    hs = {}
                    z = {}
                    for b in range(outs[-1], -1, -1):
                        xr, xi = sf_s[b, re], sf_s[b, im]
                        for a in outs:
                            if a < b:
                                continue
                            if a - b not in hs:
                                hs[a - b] = (sf_s[NC + a - b, re], sf_s[NC + a - b, im])
                            hr, hi = hs[a - b]
                            tr = xr * hr - xi * hi
                            ti = xr * hi + xi * hr
                            z[a] = (tr, ti) if a not in z else (z[a][0] + tr, z[a][1] + ti)
                        if b == 0:
                            for a in outs:
                                for part, z0 in zip(z[a], (0, C)):
                                    z0 += (a % 4) * 2 * C + fr * 8
                                    res_s.bitcast(u32)[Z0 + a // 4, z0:z0 + 8] = pltpu.bitcast(part, u32)
                            if fr == C // 8 - 1:
                                ready.append(blk)
                        yield

        done = [0]
        pending = []

        def branch_a(blk):
            for a in range(blk * NB, (blk + 1) * NB):
                rs = slice(a * C, (a + 1) * C)
                z = pltpu.bitcast(res_s.bitcast(u32)[Z0 + a // 4, (a % 4) * 2 * C:(a % 4 + 1) * 2 * C], f32)
                re0, re1, im0, im1 = (z[n * 64:(n + 1) * 64] for n in range(4))
                for par, zz in enumerate(((re0 + re1, im0 - im1), (re0 - re1, im0 + im1))):
                    a_s[pl.ds(a * C + par, C // 2, stride=2), :] = _dot(
                        _ld(g_w, (), par * C // 2, C // 2), jnp.concatenate(zz, axis=0).astype(bf16))
                y = a_s[rs, :] * (1.0 / C) + _ld(res_s, (KV,), a * C, C).astype(f32) * dsel
                xq = pltpu.bitcast(x_w[a * C // 2:(a + 1) * C // 2, col], bf16).astype(f32)
                av = gate_s[rs, :] * (xq * y)
                if a * C // TQ in pending:
                    o_b[slot, rs, :] = (av + b_s[rs, :]).astype(bf16)
                    if (a + 1) * C % TQ == 0:
                        pending.remove(a * C // TQ)
                else:
                    a_s[rs, :] = av
                done[0] = (a + 1) * C

        NG = H // HG
        SL = TQ // 32
        state = dict(prev=last, points=0, conv=0, short=0)
        sgen, cgen = short_steps(), conv_steps()
        nconv = (C // 8) * sum((blk + 1) * NB for blk in range(NC // NB))
        nshort = S // SR

        def out_proj(r):
            acc = None
            for g in range(NG):
                parts = []
                for i in range(SL):
                    mark = state["prev"][32 * i:32 * i + 8]
                    if r == 0:
                        want = min(nshort, -(-(g * SL + i + 1) * nshort // ((NG - 1) * SL)))
                        if want > state["short"]:
                            akv_w[slot + zero, 2, 0:8] = pltpu.bitcast(mark, u32)
                            while state["short"] < want:
                                next(sgen)
                                state["short"] += 1
                    elif r > 1 or g >= 1:
                        state["points"] += 1
                        want = min(nconv, -(-state["points"] * nconv // (NWIN * SL)))
                        if want > state["conv"]:
                            sf_s[2 * NC + zero, 0:8] = mark
                            while state["conv"] < want:
                                next(cgen)
                                state["conv"] += 1
                    parts.append(jnp.concatenate(
                        [_ld(res_s, (h,), r * TQ + 32 * i, 32) for h in range(g * HG, (g + 1) * HG)], axis=1))
                t = _dot(jnp.concatenate(parts, axis=0), _ld(wo_w, (slot,), g * HG * DH, HG * DH))
                state["prev"] = t
                acc = t if acc is None else acc + t
                while settled:
                    branch_a(settled.pop(0))
                while ready:
                    settled.append(ready.pop(0))
            return acc

        for r in range(S // TQ):
            acc = out_proj(r)
            if r == 0:
                for a in range(NC):
                    xm = _dot(_ld(f_w, (), 0, 2 * C), _ld(res_s, (KV,), a * C, C))
                    sf_s[a + zero] = xm
                state["prev"] = xm
            rs = slice(r * TQ, (r + 1) * TQ)
            if done[0] >= (r + 1) * TQ:
                o_b[slot, rs, :] = (a_s[rs, :] + (1.0 - gate_s[rs, :]) * acc).astype(bf16)
            else:
                b_s[rs, :] = (1.0 - gate_s[rs, :]) * acc
                pending.append(r)
        assert not pending and state["conv"] == nconv and state["short"] == nshort
        out_copy(j, slot).start()
        return carry

    lax.fori_loop(0, NDT, mix, 0)
    out_copy(NDT - 2, 0).wait()
    out_copy(NDT - 1, 1).wait()


@jax.jit
def pallas_gated_mix__ssm_conv_h3__compressed_kv_cla__prompt_kernel(
    A_q: jax.Array,
    A_k: jax.Array,
    A_v: jax.Array,
    A_shift_k: jax.Array,
    A_ssm_k: jax.Array,
    A_ssm_D: jax.Array,
    B_x: jax.Array,
    B_c_kv: jax.Array,
    B_w_q: jax.Array,
    B_w_uk: jax.Array,
    B_w_uv: jax.Array,
    B_w_o: jax.Array,
    gate_w: jax.Array,
):
    del B_x
    fwd, inv = _dft_matrices()
    V = pltpu.VMEM
    dma = pltpu.SemaphoreType.DMA
    out = pl.pallas_call(
        _kernel,
        in_specs=[pl.BlockSpec(memory_space=pl.ANY)] * 14,
        out_specs=pl.BlockSpec(memory_space=pl.ANY),
        out_shape=jax.ShapeDtypeStruct((S, M), bf16),
        scratch_shapes=[
            V((S // 2, M), u32), V((S // 2, DC), u32),
            V((2, M, DH), u32), V((2, DC, DH), u32), V((2, DC, DH), u32),
            V((2, H * DH // 2, C), u32), V((2, 3, S // 2, C), u32),
            V((2, C // 2, S), u32), V((2, S, C), bf16),
            V((4, M), bf16), V((M,), bf16), V((M,), bf16),
            V((C, C), u32), V((C // 2, C), u32),
            V((TQ, DH), bf16), V((TQ, DH), bf16), V((NC, DH, C), bf16), V((S, DH), bf16),
            V((H + 6, S, DH), bf16), V((S, C), f32), V((8, C), f32),
            V((2 * NC + 1, 2 * C, C), f32), V((S, C), f32), V((S, C), f32),
            dma((5,)), dma((2, S // TQ)), dma((3, 2)), dma((4, 2)), dma((2,)),
        ],
        compiler_params=pltpu.CompilerParams(vmem_limit_bytes=100 * 1024 * 1024),
        name="fused",
    )(A_q.reshape(S, M), B_c_kv.reshape(S, DC), B_w_q, B_w_uk, B_w_uv, B_w_o.reshape(H * DH, M),
      A_k.reshape(S, M), A_v.reshape(S, M), A_shift_k.T, A_ssm_k, A_ssm_D, gate_w,
      fwd.astype(bf16), inv.astype(bf16))
    return out.reshape(1, S, M)
```
